```python
import os as _os
_os.environ.setdefault("JAX_PLATFORMS", "cpu")
import jax
import jax.numpy as jnp

def _softmax(x, axis=-1):
    return jax.nn.softmax(x, axis=axis)
def _gelu(x):
    return jax.nn.gelu(x, approximate=True)
def _silu(x):
    return jax.nn.silu(x)
def _sigmoid(x):
    return jax.nn.sigmoid(x)
def _layernorm(x, axis=-1, eps=1e-5):
    m = jnp.mean(x, axis=axis, keepdims=True)
    v = jnp.var(x, axis=axis, keepdims=True)
    return (x - m) / jnp.sqrt(v + eps)
def _scatter_add(tgt, idx, src, axis=0):
    return tgt.at[idx].add(src)
def _segment_sum(src, seg, n):
    return jax.ops.segment_sum(src, seg, n)
class _Rng:
    def __init__(self, key):
        self._k = key
    def _next(self):
        self._k, sub = jax.random.split(self._k)
        return sub
    def normal(self, shape):
        return jax.random.normal(self._next(), shape, dtype=jnp.bfloat16)
    def randint(self, lo, hi, shape):
        return jax.random.randint(self._next(), shape, lo, hi, dtype=jnp.int32)
    def uniform(self, shape, lo=0.0, hi=1.0):
        return jax.random.uniform(self._next(), shape, jnp.bfloat16, lo, hi)
    def permutation(self, n):
        return jax.random.permutation(self._next(), n)


kernel_name = 'sequential_preLN__linear_kernel_hedgehog__geglu_ffn__prompt'

def setup_inputs():
    _rng = _Rng(jax.random.key(int.from_bytes(__import__("os").urandom(4), "little")))
    _w = (lambda a: (lambda t: t.astype(jnp.bfloat16) if jnp.issubdtype(t.dtype, jnp.floating) else t)(jnp.asarray(a)))
    def _A_setup():
        B, S, D, H = 1, 2048, 640, 32
        Dh = D // H
        return {
            "x": _w((lambda *s: _rng.normal(s) * 0.05)(B, S, D)),
            "wqkv": _w((lambda *s: _rng.normal(s) * 0.2)(D, 3 * D)),
            "w_phi": _w((lambda *s: _rng.normal(s) * 0.2)(H, Dh, Dh) * (Dh ** -0.5)),
            "wo": _w((lambda *s: _rng.normal(s) * 0.05)(D, D)),
        }
    _A_in = _A_setup()

    def _B_setup():
        B, S, D, F = 1, 2048, 640, 1536
        return {
            "x": _w((lambda *s: _rng.normal(s) * 0.05)(B, S, D)),
            "w_gate": _w((lambda *s: _rng.normal(s) * 0.05)(D, F)),
            "w_up": _w((lambda *s: _rng.normal(s) * 0.05)(D, F)),
            "w_down": _w((lambda *s: _rng.normal(s) * 0.05)(F, D)),
        }
    _B_in = _B_setup()

    return {
        "A_x": _A_in["x"],
        "A_wqkv": _A_in["wqkv"],
        "A_w_phi": _A_in["w_phi"],
        "A_wo": _A_in["wo"],
        "B_x": _B_in["x"],
        "B_w_gate": _B_in["w_gate"],
        "B_w_up": _B_in["w_up"],
        "B_w_down": _B_in["w_down"],
    }

def reference(A_x, A_wqkv, A_w_phi, A_wo, B_x, B_w_gate, B_w_up, B_w_down):
    def _A_ref(x, wqkv, w_phi, wo):
        B, S, D = x.shape
        H = 32; Dh = D // H
        qkv = (lambda x, *d: x.transpose(*d))((x @ wqkv).reshape(B, S, 3, H, Dh), 2, 0, 3, 1, 4)
        q, k, v = qkv[0], qkv[1], qkv[2]
        pq = jnp.einsum("bhsd,hdf->bhsf", q, w_phi)
        pk = jnp.einsum("bhsd,hdf->bhsf", k, w_phi)
        phi_q = jnp.concatenate([_softmax(pq, axis=-1), _softmax(-pq, axis=-1)], axis=-1)
        phi_k = jnp.concatenate([_softmax(pk, axis=-1), _softmax(-pk, axis=-1)], axis=-1)
        kv = jnp.einsum("bhsf,bhsd->bhfd", phi_k, v)
        z  = jnp.einsum("bhsf->bhf", phi_k)
        num = jnp.einsum("bhqf,bhfd->bhqd", phi_q, kv)
        den = jnp.einsum("bhqf,bhf->bhq", phi_q, z)[..., None] + 1e-6
        o = num / den
        return (lambda x, *d: x.transpose(*d))(o, 0, 2, 1, 3).reshape(B, S, D) @ wo

    def _B_ref(x, w_gate, w_up, w_down):
        return (_gelu(x @ w_gate) * (x @ w_up)) @ w_down

    x = A_x
    h = x + _A_ref(_layernorm(x, axis=-1), A_wqkv, A_w_phi, A_wo)
    h2 = h + _B_ref(_layernorm(h, axis=-1), B_w_gate, B_w_up, B_w_down)
    return h2
```

```python
import functools
import numpy as np
import jax
import jax.numpy as jnp
from jax import lax
import jax.experimental.pallas as pl
import jax.experimental.pallas.tpu as pltpu

H = 32
HG = 2
LOG2E = float(np.log2(np.e))
NT = (((1,), (1,)), ((), ()))
F32 = jnp.float32
BF16 = jnp.bfloat16
U32 = jnp.uint32


def _scope(name, on):
    import contextlib
    return jax.named_scope(name) if on else contextlib.nullcontext()


def _pack(x):
    return pltpu.bitcast(x.astype(BF16), U32)


def _unpack(x):
    return pltpu.bitcast(x, BF16)


def _layernorm(x):
    m = jnp.mean(x, axis=-1, keepdims=True)
    d = x - m
    v = jnp.mean(d * d, axis=-1, keepdims=True)
    return d * lax.rsqrt(v + 1e-5)


def _gelu(x):
    c0 = float(np.sqrt(2.0 / np.pi))
    c1 = c0 * 0.044715
    return (0.5 * x) * (1.0 + jnp.tanh(x * (c0 + c1 * (x * x))))


def _tree(op, xs):
    xs = list(xs)
    while len(xs) > 1:
        xs = [op(xs[i], xs[i + 1]) if i + 1 < len(xs) else xs[i] for i in range(0, len(xs), 2)]
    return xs[0]


def _recip(s, newton):
    if not newton:
        return 1.0 / s
    r = pl.reciprocal(s, approx=True)
    return r * (2.0 - s * r)


def _feature_map(p, newton):
    n = p.shape[0] // 8
    rows = [p[8 * j:8 * j + 8] for j in range(n)]

    def reduce(op, xs):
        y = _tree(op, xs)
        s = 4
        while s >= HG:
            y = op(y, pltpu.roll(y, s, 0))
            s //= 2
        return y

    mx = reduce(jnp.maximum, rows)
    mn = reduce(jnp.minimum, rows)
    ep = [jnp.exp2(r - mx) for r in rows]
    en = [jnp.exp2(mn - r) for r in rows]
    rp = _recip(reduce(jnp.add, ep), newton)
    rn = _recip(reduce(jnp.add, en), newton)
    return jnp.concatenate([e * rp for e in ep] + [e * rn for e in en], axis=0)


def _kernel(x_hbm, wqkv_hbm, wphi_hbm, wo_hbm, wg_hbm, wu_hbm, wd_hbm, out_hbm,
            x_v, wqkv_v, wphi_v, wo_v, wg_v, wu_v, wd_v,
            arep_v, xn_v, kt_v, wt_v, phi_v, kv_v, m_v, o_v, xsem, wsem, osem,
            *, T, FC, SP, SE, SG, NW, OPQ, TB, SC):
    S, D = x_v.shape
    F = wg_v.shape[1]
    Dh = D // H
    NG = H // HG
    GR = HG * Dh
    ZR = 4 * HG
    nT = S // T
    LHG = HG.bit_length() - 1
    DP = D // 2

    def x_copy(i):
        rows = pl.ds(pl.multiple_of(i * T, T), T)
        return pltpu.make_async_copy(x_hbm.at[rows], x_v.at[rows], xsem.at[i])

    def qkv_copy(j):
        return pltpu.make_async_copy(wqkv_hbm.at[:, pl.ds(j * D, D)], wqkv_v.at[:, pl.ds(j * D, D)], wsem.at[j])

    c_phi = pltpu.make_async_copy(wphi_hbm, wphi_v, wsem.at[3])
    c_wo = pltpu.make_async_copy(wo_hbm, wo_v, wsem.at[4])
    c_wg = pltpu.make_async_copy(wg_hbm, wg_v, wsem.at[5])
    c_wu = pltpu.make_async_copy(wu_hbm, wu_v, wsem.at[6])
    c_wd = pltpu.make_async_copy(wd_hbm, wd_v, wsem.at[7])

    def out_copy(i, slot):
        return pltpu.make_async_copy(o_v.at[slot], out_hbm.at[pl.ds(pl.multiple_of(i * T, T), T)], osem.at[slot])

    c_phi.start()
    qkv_copy(1).start()

    kv_v[...] = jnp.zeros(kv_v.shape, F32)
    c_phi.wait()
    x_copy(0).start()
    b = jnp.concatenate([wphi_v[d].astype(F32) for d in range(Dh)], axis=1)
    b = jnp.concatenate([b, jnp.zeros((32 - Dh, D), F32)], axis=0).astype(BF16)
    pr = lax.broadcasted_iota(jnp.int32, (D, D), 0)
    pc = lax.broadcasted_iota(jnp.int32, (D, D), 1)
    perm = jnp.where(pc == (pr & (H - 1)) * Dh + (pr >> 5), 1.0, 0.0).astype(BF16)
    a = jnp.dot(b, perm, preferred_element_type=F32).astype(BF16)
    r = lax.broadcasted_iota(jnp.int32, (GR, 128), 0)
    c = lax.broadcasted_iota(jnp.int32, (GR, 128), 1)
    sel = jnp.where((r >> LHG) == c, 1.0, 0.0).astype(BF16)[:, 0:32]
    arep_v[...] = jnp.dot(sel, a, preferred_element_type=F32)

    def fold(src):
        r = lax.broadcasted_iota(jnp.int32, (GR, 128), 0)
        c = lax.broadcasted_iota(jnp.int32, (GR, 128), 1)
        acc = [None] * NG
        for j in range(D // 128):
            gs = [g for g in range(NG) if g * GR < (j + 1) * 128 and (g + 1) * GR > j * 128]
            blocks = []
            for g in gs:
                lo = (HG * g + (r & (HG - 1))) * Dh - j * 128
                blocks.append(jnp.where((c >= lo) & (c < lo + Dh), arep_v[:, j * 128:(j + 1) * 128], 0.0))
            lhs = jnp.concatenate(blocks, axis=0).astype(BF16)
            res = lax.dot_general(lhs, wqkv_v[:, src * D + j * 128:src * D + (j + 1) * 128], NT,
                                  preferred_element_type=F32)
            for n, g in enumerate(gs):
                part = res[n * GR:(n + 1) * GR]
                acc[g] = part if acc[g] is None else acc[g] + part
        wt_v[src * DP:(src + 1) * DP, :] = _pack(jnp.concatenate(acc, axis=0) * LOG2E)

    def proj(src, xn):
        return lax.dot_general(_unpack(wt_v[src * DP:(src + 1) * DP, :]), xn, NT, preferred_element_type=F32)

    def k_proj(i):
        rows = pl.ds(pl.multiple_of(i * T, T), T)
        xn = _layernorm(x_v[rows, :].astype(F32)).astype(BF16)
        xn_v[...] = _pack(xn)
        kt_v[...] = proj(1, xn)

    def tile1(i, last):
        xn = _unpack(xn_v[...])
        ones = jnp.ones((ZR, T), F32)
        qT = proj(0, xn)
        for g in range(NG):
            phi_v[nT, g * GR:(g + 1) * GR, :] = _pack(_feature_map(kt_v[g * GR:(g + 1) * GR, :], NW))
        vT = proj(2, xn)
        for g in range(NG):
            phi_v[i, g * GR:(g + 1) * GR, :] = _pack(_feature_map(qT[g * GR:(g + 1) * GR], NW))
        for g in range(NG):
            vext = jnp.concatenate([vT[g * GR:(g + 1) * GR], ones], axis=0).astype(BF16)
            kv_v[g] += lax.dot_general(vext, _unpack(phi_v[nT, g * GR:(g + 1) * GR, :]), NT,
                                       preferred_element_type=F32)
        if not last:
            k_proj(i + 1)

    with _scope('w_k', SC):
        qkv_copy(1).wait()
    qkv_copy(2).start()
    with _scope('fold_k', SC):
        fold(1)
    qkv_copy(0).start()
    with _scope('w_x', SC):
        x_copy(0).wait()
    x_copy(1).start()
    with _scope('k0', SC):
        k_proj(0)
    with _scope('w_vq', SC):
        qkv_copy(2).wait()
        qkv_copy(0).wait()
    for i in range(2, nT):
        x_copy(i).start()
    c_wo.start()
    c_wg.start()
    c_wu.start()
    c_wd.start()
    with _scope('fold_q', SC):
        if TB:
            wt_v[2 * DP:3 * DP, :] = _pack(wqkv_v[:, 2 * D:3 * D].T)
        else:
            wt_v[2 * DP:3 * DP, :] = _pack(wqkv_v[:, 2 * D:3 * D].astype(F32).T)
        fold(0)

    def phase1(i, carry):
        x_copy(i + 1).wait()
        tile1(i, False)
        return carry + 1

    with _scope('phase1', SC):
        last = lax.fori_loop(0, nT - 1, phase1, 0)
    with _scope('phase1_last', SC):
        tile1(last if OPQ else nT - 1, True)

    rr = lax.broadcasted_iota(jnp.int32, (GR + ZR, 2 * GR), 0)
    cc = lax.broadcasted_iota(jnp.int32, (GR + ZR, 2 * GR), 1)
    head = jnp.where(rr < GR, sum((rr >= k * Dh).astype(jnp.int32) for k in range(1, HG)), (rr - GR) >> 2)
    keep = head == (cc & (HG - 1))
    for g in range(NG):
        m_v[g] = _pack(jnp.where(keep, kv_v[g], 0.0))

    with _scope('w_rest', SC):
        c_wo.wait()
        c_wg.wait()
        c_wu.wait()
        c_wd.wait()

    def phase2(i, carry):
        slot = i % 2

        @pl.when(i >= 2)
        def _():
            out_copy(i - 2, slot).wait()

        lo = lax.broadcasted_iota(jnp.int32, (8, T), 0) < 4
        outs = []
        for g in range(NG):
            nd = jnp.dot(_unpack(m_v[g]), _unpack(phi_v[i, g * GR:(g + 1) * GR, :]), preferred_element_type=F32)
            rec = []
            for p in range(HG // 2):
                ra = 1.0 / (nd[GR + 8 * p:GR + 8 * p + 8] + 1e-6)
                ras = pltpu.roll(ra, 4, 0)
                r0 = jnp.where(lo, ra, ras)
                r1 = jnp.where(lo, ras, ra)
                rec += [r0, r0, ra, r1, r1]
            outs.append(nd[0:GR] * jnp.concatenate(rec, axis=0))
        oT = jnp.concatenate(outs, axis=0)
        if TB:
            o = oT.astype(BF16).T
        else:
            o = oT.T.astype(BF16)

        def glu(hn, f):
            gate = jnp.dot(hn, wg_v[:, f * FC:(f + 1) * FC], preferred_element_type=F32)
            up = jnp.dot(hn, wu_v[:, f * FC:(f + 1) * FC], preferred_element_type=F32)
            return (_gelu(gate) * up).astype(BF16)

        R = T // SP
        hs, hns, acts = [], [], []
        for u in range(SP):
            xr = x_v[pl.ds(pl.multiple_of(i * T + u * R, R), R), :]
            hs.append(xr.astype(F32) + jnp.dot(o[u * R:(u + 1) * R], wo_v[...], preferred_element_type=F32))
            hns.append(_layernorm(hs[u]).astype(BF16))
        hn = jnp.concatenate(hns, axis=0)
        if SG:
            act = jnp.concatenate([glu(hns[u], 0) for u in range(SP)], axis=0)
        else:
            act = glu(hn, 0)
        acc = jnp.concatenate(hs, axis=0)
        nF = F // FC
        for f in range(1, nF):
            nxt = glu(hn, f)
            acc = acc + jnp.dot(act, wd_v[(f - 1) * FC:f * FC, :], preferred_element_type=F32)
            act = nxt
        R = T // SE
        for u in range(SE):
            y = acc[u * R:(u + 1) * R] + jnp.dot(act[u * R:(u + 1) * R], wd_v[(nF - 1) * FC:nF * FC, :],
                                                 preferred_element_type=F32)
            o_v[slot, u * R:(u + 1) * R, :] = y.astype(BF16)
        out_copy(i, slot).start()
        return carry

    with _scope('phase2', SC):
        lax.fori_loop(0, nT, phase2, 0)
    with _scope('tail', SC):
        out_copy(nT - 2, (nT - 2) % 2).wait()
        out_copy(nT - 1, (nT - 1) % 2).wait()


def build(T=512, FC=512, SP=4, SE=4, SG=0, NW=1, OPQ=1, TB=0, SC=0):
    def fn(A_x, A_wqkv, A_w_phi, A_wo, B_x, B_w_gate, B_w_up, B_w_down):
        del B_x
        B, S, D = A_x.shape
        F = B_w_gate.shape[1]
        Dh = D // H
        NG = H // HG
        GR = HG * Dh
        ZR = 4 * HG
        nT = S // T
        any_spec = pl.BlockSpec(memory_space=pl.ANY)
        out = pl.pallas_call(
            functools.partial(_kernel, T=T, FC=FC, SP=SP, SE=SE, SG=SG, NW=NW, OPQ=OPQ, TB=TB, SC=SC),
            out_shape=jax.ShapeDtypeStruct((S, D), A_x.dtype),
            in_specs=[any_spec] * 7,
            out_specs=any_spec,
            scratch_shapes=[
                pltpu.VMEM((S, D), BF16),
                pltpu.VMEM((D, 3 * D), BF16),
                pltpu.VMEM((Dh, Dh, H), BF16),
                pltpu.VMEM((D, D), BF16),
                pltpu.VMEM((D, F), BF16),
                pltpu.VMEM((D, F), BF16),
                pltpu.VMEM((F, D), BF16),
                pltpu.VMEM((GR, D), F32),
                pltpu.VMEM((T // 2, D), U32),
                pltpu.VMEM((D, T), F32),
                pltpu.VMEM((3 * D // 2, D), U32),
                pltpu.VMEM((nT + 1, D, T), U32),
                pltpu.VMEM((NG, GR + ZR, 2 * GR), F32),
                pltpu.VMEM((NG, (GR + ZR) // 2, 2 * GR), U32),
                pltpu.VMEM((2, T, D), BF16),
                pltpu.SemaphoreType.DMA((nT,)),
                pltpu.SemaphoreType.DMA((8,)),
                pltpu.SemaphoreType.DMA((2,)),
            ],
            compiler_params=pltpu.CompilerParams(vmem_limit_bytes=100 * 1024 * 1024),
        )(A_x.reshape(S, D), A_wqkv, A_w_phi.transpose(1, 2, 0), A_wo, B_w_gate, B_w_up, B_w_down)
        return out.reshape(B, S, D)
    return fn


pallas_sequential_preLN__linear_kernel_hedgehog__geglu_ffn__prompt_kernel = jax.jit(build())
```

```python
import jax
import jax.numpy as jnp
import numpy as np
from jax import lax
import jax.experimental.pallas as pl
import jax.experimental.pallas.tpu as pltpu

HEADS = 32
PAIR = 2
TILE = 512
SUB = 128
FF_CHUNK = 768
WK_SPLIT = 384
LANES = 128
LOG2E = float(np.log2(np.e))
GELU_C0 = float(np.sqrt(2.0 / np.pi))
GELU_C1 = GELU_C0 * 0.044715
NT_DIMS = (((1,), (1,)), ((), ()))
F32 = jnp.float32
BF16 = jnp.bfloat16
U32 = jnp.uint32


def _to_words(x):
    return pltpu.bitcast(x.astype(BF16), U32)


def _from_words(x):
    return pltpu.bitcast(x, BF16)


def _dot(a, b):
    return jnp.dot(a, b, preferred_element_type=F32)


def _dot_nt(a, b):
    return lax.dot_general(a, b, NT_DIMS, preferred_element_type=F32)


def _iota(shape, axis):
    return lax.broadcasted_iota(jnp.int32, shape, axis)


def _layernorm(x):
    d = x - jnp.mean(x, axis=-1, keepdims=True)
    return d * lax.rsqrt(jnp.mean(d * d, axis=-1, keepdims=True) + 1e-5)


def _gelu(x):
    return (0.5 * x) * (1.0 + jnp.tanh(x * (GELU_C0 + GELU_C1 * (x * x))))


def _per_head(op, vregs):
    while len(vregs) > 1:
        vregs = [op(*vregs[i:i + 2]) if i + 1 < len(vregs) else vregs[i] for i in range(0, len(vregs), 2)]
    y = vregs[0]
    y = op(y, pltpu.roll(y, 4, 0))
    return op(y, pltpu.roll(y, 2, 0))


def _recip(s):
    r = pl.reciprocal(s, approx=True)
    return r * (2.0 - s * r)


def _feature_map(p):
    rows = [p[j:j + 8] for j in range(0, p.shape[0], 8)]
    hi = _per_head(jnp.maximum, rows)
    lo = _per_head(jnp.minimum, rows)
    pos = [jnp.exp2(r - hi) for r in rows]
    neg = [jnp.exp2(lo - r) for r in rows]
    pos_scale = _recip(_per_head(jnp.add, pos))
    neg_scale = _recip(_per_head(jnp.add, neg))
    return jnp.concatenate([e * pos_scale for e in pos] + [e * neg_scale for e in neg], axis=0)


def _kernel(x_hbm, wqkv_hbm, wphi_hbm, wo_hbm, wg_hbm, wu_hbm, wd_hbm, out_hbm,
            x_v, wq_v, wka_v, wkb_v, wv_v, wphi_v, wo_v, wg_v, wu_v, wd_v,
            band_v, wt_v, xn_v, kt_v, phi_v, state_v, read_v, out_v,
            x_sem, w_sem, out_sem):
    n_tiles, T, D = x_v.shape
    F = wg_v.shape[1]
    dh = D // HEADS
    n_groups = HEADS // PAIR
    gr = PAIR * dh
    n_sub = T // SUB
    k_tiles = D // LANES
    Q, K, V = range(3)

    def x_copy(i):
        rows = pl.ds(pl.multiple_of(i * T, T), T)
        return pltpu.make_async_copy(x_hbm.at[rows], x_v.at[i], x_sem.at[i])

    def out_copy(j):
        rows = pl.ds(pl.multiple_of(j * SUB, SUB), SUB)
        return pltpu.make_async_copy(out_v.at[j], out_hbm.at[rows], out_sem.at[j])

    half = T // 2
    first_x_copies = [
        pltpu.make_async_copy(x_hbm.at[pl.ds(lo, half)], x_v.at[0, pl.ds(lo, half)], sem)
        for lo, sem in ((0, x_sem.at[0]), (half, w_sem.at[9]))]
    wq_copy = pltpu.make_async_copy(wqkv_hbm.at[:, pl.ds(Q * D, D)], wq_v, w_sem.at[0])
    wka_copy = pltpu.make_async_copy(wqkv_hbm.at[pl.ds(0, WK_SPLIT), pl.ds(K * D, D)], wka_v, w_sem.at[1])
    wkb_copy = pltpu.make_async_copy(wqkv_hbm.at[pl.ds(WK_SPLIT, D - WK_SPLIT), pl.ds(K * D, D)], wkb_v,
                                     w_sem.at[2])
    wv_copy = pltpu.make_async_copy(wqkv_hbm.at[:, pl.ds(V * D, D)], wv_v, w_sem.at[3])
    wphi_copy = pltpu.make_async_copy(wphi_hbm, wphi_v, w_sem.at[4])
    late_copies = [pltpu.make_async_copy(src, dst, w_sem.at[5 + n]) for n, (src, dst) in enumerate(
        [(wo_hbm, wo_v), (wg_hbm, wg_v), (wu_hbm, wu_v), (wd_hbm, wd_v)])]

    wphi_copy.start()
    wka_copy.start()
    state_v[...] = jnp.zeros(state_v.shape, F32)
    wphi_copy.wait()
    wkb_copy.start()

    flat = jnp.concatenate([wphi_v[d].astype(F32) for d in range(dh)], axis=1)
    flat = jnp.concatenate([flat, jnp.zeros((HEADS - dh, D), F32)], axis=0).astype(BF16)
    src = _iota((D, D), 0)
    swap = jnp.where(_iota((D, D), 1) == (src & (HEADS - 1)) * dh + (src >> 5), 1.0, 0.0).astype(BF16)
    flat = _dot(flat, swap).astype(BF16)
    row, col = _iota((gr, LANES), 0), _iota((gr, LANES), 1)
    repeat = jnp.where((row >> 1) == col, 1.0, 0.0).astype(BF16)[:, 0:HEADS]
    flat = _dot(repeat, flat)
    overlap = [[g for g in range(n_groups) if g * gr < (j + 1) * LANES and (g + 1) * gr > j * LANES]
               for j in range(k_tiles)]
    for copy in first_x_copies:
        copy.start()
    for j in range(k_tiles):
        blocks = []
        for g in overlap[j]:
            first = (PAIR * g + (row & 1)) * dh - j * LANES
            blocks.append(jnp.where((col >= first) & (col < first + dh),
                                    flat[:, j * LANES:(j + 1) * LANES], 0.0))
        band_v[j] = _to_words(jnp.concatenate(blocks, axis=0))

    def fold(which, w_ref, lo):
        acc = [None] * n_groups
        for j in range(k_tiles):
            res = _dot_nt(_from_words(band_v[j]), w_ref[:, j * LANES:(j + 1) * LANES])
            for n, g in enumerate(overlap[j]):
                part = res[n * gr:(n + 1) * gr]
                acc[g] = part if acc[g] is None else acc[g] + part
        wt_v[which, :, lo:lo + w_ref.shape[0]] = _to_words(jnp.concatenate(acc, axis=0) * LOG2E)

    def project(which, xn):
        return _dot_nt(_from_words(wt_v[which]), xn)

    def store_phi(slot, logits):
        for g in range(n_groups):
            phi = _feature_map(logits[g * gr:(g + 1) * gr, :])
            for c in range(0, T, LANES):
                phi_v[slot, g * gr:(g + 1) * gr, c:c + LANES] = _to_words(phi[:, c:c + LANES])

    def load_phi(slot, g):
        return _from_words(phi_v[slot, g * gr:(g + 1) * gr, :])

    def start_tile(i):
        xn = _layernorm(x_v[i].astype(F32)).astype(BF16)
        xn_v[...] = _to_words(xn)
        kt_v[...] = project(K, xn)

    def finish_tile(i, start_next):
        xn = _from_words(xn_v[...])
        qt = project(Q, xn)
        store_phi(n_tiles, kt_v)
        vt = project(V, xn)
        if not start_next:
            store_phi(i, qt)
        ones = jnp.ones((8, T), F32)
        for g in range(n_groups):
            v_ones = jnp.concatenate([vt[g * gr:(g + 1) * gr], ones], axis=0).astype(BF16)
            state_v[g] += _dot_nt(v_ones, load_phi(n_tiles, g))
        if start_next:
            start_tile(i + 1)
            store_phi(i, qt)

    wka_copy.wait()
    fold(K, wka_v, 0)
    wkb_copy.wait()
    wv_copy.start()
    wq_copy.start()
    fold(K, wkb_v, WK_SPLIT)
    for n, copy in enumerate(first_x_copies):
        copy.wait()
        xn = _layernorm(x_v[0, n * half:(n + 1) * half, :].astype(F32))
        xn_v[n * half // 2:(n + 1) * half // 2, :] = _to_words(xn)
    kt_v[...] = project(K, _from_words(xn_v[...]))
    x_copy(1).start()
    wv_copy.wait()
    wq_copy.wait()
    for i in range(2, n_tiles):
        x_copy(i).start()
    for copy in late_copies:
        copy.start()
    wt_v[V] = _to_words(wv_v[...].T)
    fold(Q, wq_v, 0)

    def pass1(i, count):
        x_copy(i + 1).wait()
        finish_tile(i, True)
        return count + 1

    finish_tile(lax.fori_loop(0, n_tiles - 1, pass1, 0), False)

    row, col = _iota((gr + 8, 2 * gr), 0), _iota((gr + 8, 2 * gr), 1)
    head = jnp.where(row < gr, (row >= dh).astype(jnp.int32), (row - gr) >> 2)
    own = head == (col & 1)
    for g in range(n_groups):
        read_v[g] = _to_words(jnp.where(own, state_v[g], 0.0))
    for copy in late_copies:
        copy.wait()

    def glu(hn, c):
        cols = slice(c * FF_CHUNK, (c + 1) * FF_CHUNK)
        return (_gelu(_dot(hn, wg_v[:, cols])) * _dot(hn, wu_v[:, cols])).astype(BF16)

    def pass2(i, carry):
        first_head = _iota((8, T), 0) < 4
        parts = []
        for g in range(n_groups):
            num_den = _dot(_from_words(read_v[g]), load_phi(i, g))
            both = 1.0 / (num_den[gr:gr + 8] + 1e-6)
            swapped = pltpu.roll(both, 4, 0)
            inv0 = jnp.where(first_head, both, swapped)
            inv1 = jnp.where(first_head, swapped, both)
            parts.append(num_den[0:gr] * jnp.concatenate([inv0, inv0, both, inv1, inv1], axis=0))
        o = jnp.concatenate(parts, axis=0).astype(BF16).T

        hs, hns = [], []
        for u in range(n_sub):
            rows = slice(u * SUB, (u + 1) * SUB)
            hs.append(x_v[i, rows, :].astype(F32) + _dot(o[rows], wo_v[...]))
            hns.append(_layernorm(hs[u]).astype(BF16))
        hn = jnp.concatenate(hns, axis=0)
        acc = jnp.concatenate(hs, axis=0)
        act = glu(hn, 0)
        n_chunks = F // FF_CHUNK
        for c in range(1, n_chunks):
            nxt = glu(hn, c)
            acc = acc + _dot(act, wd_v[(c - 1) * FF_CHUNK:c * FF_CHUNK, :])
            act = nxt
        for u in range(n_sub):
            rows = slice(u * SUB, (u + 1) * SUB)
            y = acc[rows] + _dot(act[rows], wd_v[F - FF_CHUNK:F, :])
            out_v[i * n_sub + u] = y.astype(BF16)
            out_copy(i * n_sub + u).start()
        return carry

    lax.fori_loop(0, n_tiles, pass2, 0)
    for j in range(n_tiles * n_sub):
        out_copy(j).wait()


def build(interpret=False):
    def fn(A_x, A_wqkv, A_w_phi, A_wo, B_x, B_w_gate, B_w_up, B_w_down):
        del B_x
        B, S, D = A_x.shape
        F = B_w_gate.shape[1]
        dh = D // HEADS
        gr = PAIR * dh
        n_tiles = S // TILE
        assert B == 1 and dh == 20 and S % TILE == 0 and n_tiles >= 2 and F % FF_CHUNK == 0
        hbm = pl.BlockSpec(memory_space=pl.ANY)
        out = pl.pallas_call(
            _kernel,
            out_shape=jax.ShapeDtypeStruct((S, D), A_x.dtype),
            in_specs=[hbm] * 7,
            out_specs=hbm,
            scratch_shapes=[
                pltpu.VMEM((n_tiles, TILE, D), BF16),
                pltpu.VMEM((D, D), BF16),
                pltpu.VMEM((WK_SPLIT, D), BF16),
                pltpu.VMEM((D - WK_SPLIT, D), BF16),
                pltpu.VMEM((D, D), BF16),
                pltpu.VMEM((dh, dh, HEADS), BF16),
                pltpu.VMEM((D, D), BF16),
                pltpu.VMEM((D, F), BF16),
                pltpu.VMEM((D, F), BF16),
                pltpu.VMEM((F, D), BF16),
                pltpu.VMEM((D // LANES, 2 * gr, LANES), U32),
                pltpu.VMEM((3, D // 2, D), U32),
                pltpu.VMEM((TILE // 2, D), U32),
                pltpu.VMEM((D, TILE), F32),
                pltpu.VMEM((n_tiles + 1, D, TILE), U32),
                pltpu.VMEM((HEADS // PAIR, gr + 8, 2 * gr), F32),
                pltpu.VMEM((HEADS // PAIR, gr // 2 + 4, 2 * gr), U32),
                pltpu.VMEM((S // SUB, SUB, D), BF16),
                pltpu.SemaphoreType.DMA((n_tiles,)),
                pltpu.SemaphoreType.DMA((10,)),
                pltpu.SemaphoreType.DMA((S // SUB,)),
            ],
            compiler_params=pltpu.CompilerParams(vmem_limit_bytes=100 * 1024 * 1024),
            interpret=interpret,
        )(A_x.reshape(S, D), A_wqkv, A_w_phi.transpose(1, 2, 0), A_wo, B_w_gate, B_w_up, B_w_down)
        return out.reshape(B, S, D)
    return fn


pallas_sequential_preLN__linear_kernel_hedgehog__geglu_ffn__prompt_kernel = jax.jit(build())
```

```python
import jax
import jax.numpy as jnp
import numpy as np
from jax import lax
import jax.experimental.pallas as pl
import jax.experimental.pallas.tpu as pltpu

HEADS = 32
PAIR = 2
TILE = 512
WO_ROWS = 64
OUT_ROWS = 128
FF_CHUNK = 256
WK_SPLIT = 384
LANES = 128
LOG2E = float(np.log2(np.e))
GELU_C0 = float(np.sqrt(2.0 / np.pi))
GELU_C1 = GELU_C0 * 0.044715
NT_DIMS = (((1,), (1,)), ((), ()))
F32 = jnp.float32
BF16 = jnp.bfloat16
U32 = jnp.uint32


def _to_words(x):
    return pltpu.bitcast(x.astype(BF16), U32)


def _from_words(x):
    return pltpu.bitcast(x, BF16)


def _dot(a, b):
    return jnp.dot(a, b, preferred_element_type=F32)


def _dot_nt(a, b):
    return lax.dot_general(a, b, NT_DIMS, preferred_element_type=F32)


def _iota(shape, axis):
    return lax.broadcasted_iota(jnp.int32, shape, axis)


def _layernorm(x):
    d = x - jnp.mean(x, axis=-1, keepdims=True)
    return d * lax.rsqrt(jnp.mean(d * d, axis=-1, keepdims=True) + 1e-5)


def _gelu(x):
    return (0.5 * x) * (1.0 + jnp.tanh(x * (GELU_C0 + GELU_C1 * (x * x))))


def _per_head(op, vregs):
    while len(vregs) > 1:
        vregs = [op(*vregs[i:i + 2]) if i + 1 < len(vregs) else vregs[i] for i in range(0, len(vregs), 2)]
    y = vregs[0]
    y = op(y, pltpu.roll(y, 4, 0))
    return op(y, pltpu.roll(y, 2, 0))


def _recip(s):
    r = pl.reciprocal(s, approx=True)
    return r * (2.0 - s * r)


def _feature_map(p):
    rows = [p[j:j + 8] for j in range(0, p.shape[0], 8)]
    hi = _per_head(jnp.maximum, rows)
    lo = _per_head(jnp.minimum, rows)
    pos = [jnp.exp2(r - hi) for r in rows]
    neg = [jnp.exp2(lo - r) for r in rows]
    pos_scale = _recip(_per_head(jnp.add, pos))
    neg_scale = _recip(_per_head(jnp.add, neg))
    return jnp.concatenate([e * pos_scale for e in pos] + [e * neg_scale for e in neg], axis=0)


def _strassen_lhs(a11, a12, a21, a22):
    return [a11 + a22, a21 + a22, a11, a22, a11 + a12, a21 - a11, a12 - a22]


def _strassen_rhs(b11, b12, b21, b22):
    return [b11 + b22, b11, b12 - b22, b21 - b11, b22, b11 + b12, b21 + b22]


RHS_SUMS = (0, 2, 3, 5, 6)


def _strassen_out(m):
    return (m[0] + m[3]) + (m[6] - m[4]), m[2] + m[4], m[1] + m[3], (m[0] - m[1]) + (m[2] + m[5])


def _kernel(x_hbm, wqkv_hbm, wphi_hbm, wo_hbm, wg_hbm, wu_hbm, wd_hbm, out_hbm,
            x_v, wq_v, wka_v, wkb_v, wv_v, wphi_v, wo_v, wg_v, wu_v, wd_v,
            gate_up_sums_v, down_sums_v, band_v, wt_v, xn_v, kt_v, phi_v, state_v, read_v, out_v,
            x_sem, w_sem, out_sem):
    n_tiles, T, D = x_v.shape
    F = wg_v.shape[1]
    dh = D // HEADS
    n_groups = HEADS // PAIR
    gr = PAIR * dh
    n_out = T // OUT_ROWS
    n_chunks = F // FF_CHUNK
    th, dq, fh = T // 2, 2 * LANES, FF_CHUNK // 2
    k_tiles = D // LANES
    Q, K, V = range(3)

    def x_copy(i):
        rows = pl.ds(pl.multiple_of(i * T, T), T)
        return pltpu.make_async_copy(x_hbm.at[rows], x_v.at[i], x_sem.at[i])

    def out_copy(j):
        rows = pl.ds(pl.multiple_of(j * OUT_ROWS, OUT_ROWS), OUT_ROWS)
        return pltpu.make_async_copy(out_v.at[j], out_hbm.at[rows], out_sem.at[j])

    half = T // 2
    first_x_copies = [
        pltpu.make_async_copy(x_hbm.at[pl.ds(lo, half)], x_v.at[0, pl.ds(lo, half)], sem)
        for lo, sem in ((0, x_sem.at[0]), (half, w_sem.at[9]))]
    wq_copy = pltpu.make_async_copy(wqkv_hbm.at[:, pl.ds(Q * D, D)], wq_v, w_sem.at[0])
    wka_copy = pltpu.make_async_copy(wqkv_hbm.at[pl.ds(0, WK_SPLIT), pl.ds(K * D, D)], wka_v, w_sem.at[1])
    wkb_copy = pltpu.make_async_copy(wqkv_hbm.at[pl.ds(WK_SPLIT, D - WK_SPLIT), pl.ds(K * D, D)], wkb_v,
                                     w_sem.at[2])
    wv_copy = pltpu.make_async_copy(wqkv_hbm.at[:, pl.ds(V * D, D)], wv_v, w_sem.at[3])
    wphi_copy = pltpu.make_async_copy(wphi_hbm, wphi_v, w_sem.at[4])
    late_copies = [pltpu.make_async_copy(src, dst, w_sem.at[5 + n]) for n, (src, dst) in enumerate(
        [(wo_hbm, wo_v), (wg_hbm, wg_v), (wu_hbm, wu_v), (wd_hbm, wd_v)])]

    wphi_copy.start()
    wka_copy.start()
    state_v[...] = jnp.zeros(state_v.shape, F32)
    wphi_copy.wait()
    wkb_copy.start()

    flat = jnp.concatenate([wphi_v[d].astype(F32) for d in range(dh)], axis=1)
    flat = jnp.concatenate([flat, jnp.zeros((HEADS - dh, D), F32)], axis=0).astype(BF16)
    src = _iota((D, D), 0)
    swap = jnp.where(_iota((D, D), 1) == (src & (HEADS - 1)) * dh + (src >> 5), 1.0, 0.0).astype(BF16)
    flat = _dot(flat, swap).astype(BF16)
    row, col = _iota((gr, LANES), 0), _iota((gr, LANES), 1)
    repeat = jnp.where((row >> 1) == col, 1.0, 0.0).astype(BF16)[:, 0:HEADS]
    flat = _dot(repeat, flat)
    overlap = [[g for g in range(n_groups) if g * gr < (j + 1) * LANES and (g + 1) * gr > j * LANES]
               for j in range(k_tiles)]
    for copy in first_x_copies:
        copy.start()
    for j in range(k_tiles):
        blocks = []
        for g in overlap[j]:
            first = (PAIR * g + (row & 1)) * dh - j * LANES
            blocks.append(jnp.where((col >= first) & (col < first + dh),
                                    flat[:, j * LANES:(j + 1) * LANES], 0.0))
        band_v[j] = _to_words(jnp.concatenate(blocks, axis=0))

    def fold(which, w_ref, lo):
        acc = [None] * n_groups
        for j in range(k_tiles):
            res = _dot_nt(_from_words(band_v[j]), w_ref[:, j * LANES:(j + 1) * LANES])
            for n, g in enumerate(overlap[j]):
                part = res[n * gr:(n + 1) * gr]
                acc[g] = part if acc[g] is None else acc[g] + part
        wt_v[which, :, lo:lo + w_ref.shape[0]] = _to_words(jnp.concatenate(acc, axis=0) * LOG2E)

    def project(which, xn):
        return _dot_nt(_from_words(wt_v[which]), xn)

    def store_phi(slot, logits):
        for g in range(n_groups):
            phi = _feature_map(logits[g * gr:(g + 1) * gr, :])
            for c in range(0, T, LANES):
                phi_v[slot, g * gr:(g + 1) * gr, c:c + LANES] = _to_words(phi[:, c:c + LANES])

    def load_phi(slot, g):
        return _from_words(phi_v[slot, g * gr:(g + 1) * gr, :])

    def store_block_sums(w_ref, r0, rn, c0, cn, dst):
        for r in range(0, rn, 16):
            ops = _strassen_rhs(*[
                w_ref[r0 + a * rn + r:r0 + a * rn + r + 16, c0 + b * cn:c0 + (b + 1) * cn].astype(F32)
                for a in range(2) for b in range(2)])
            for n, j in enumerate(RHS_SUMS):
                dst[n, r:r + 16, :] = ops[j].astype(BF16)

    def prepare_ffn_weights():
        for c in range(n_chunks):
            store_block_sums(wg_v, 0, dq, c * FF_CHUNK, fh, gate_up_sums_v.at[c, :, :, 0:fh])
            store_block_sums(wu_v, 0, dq, c * FF_CHUNK, fh, gate_up_sums_v.at[c, :, :, fh:FF_CHUNK])
            store_block_sums(wd_v, c * FF_CHUNK, fh, 0, dq, down_sums_v.at[c])

    def start_tile(i):
        xn = _layernorm(x_v[i].astype(F32)).astype(BF16)
        xn_v[...] = _to_words(xn)
        kt_v[...] = project(K, xn)

    def finish_tile(i, start_next):
        xn = _from_words(xn_v[...])
        if not start_next:
            prepare_ffn_weights()
        qt = project(Q, xn)
        store_phi(n_tiles, kt_v)
        vt = project(V, xn)
        if not start_next:
            store_phi(i, qt)
        ones = jnp.ones((8, T), F32)
        for g in range(n_groups):
            v_ones = jnp.concatenate([vt[g * gr:(g + 1) * gr], ones], axis=0).astype(BF16)
            state_v[g] += _dot_nt(v_ones, load_phi(n_tiles, g))
        if start_next:
            start_tile(i + 1)
            store_phi(i, qt)

    wka_copy.wait()
    fold(K, wka_v, 0)
    wkb_copy.wait()
    wv_copy.start()
    wq_copy.start()
    fold(K, wkb_v, WK_SPLIT)
    for n, copy in enumerate(first_x_copies):
        copy.wait()
        xn = _layernorm(x_v[0, n * half:(n + 1) * half, :].astype(F32))
        xn_v[n * half // 2:(n + 1) * half // 2, :] = _to_words(xn)
    kt_v[...] = project(K, _from_words(xn_v[...]))
    x_copy(1).start()
    wv_copy.wait()
    wq_copy.wait()
    for i in range(2, n_tiles):
        x_copy(i).start()
    for copy in late_copies:
        copy.start()
    wt_v[V] = _to_words(wv_v[...].T)
    fold(Q, wq_v, 0)

    def pass1(i, count):
        x_copy(i + 1).wait()
        finish_tile(i, True)
        return count + 1

    last_tile = lax.fori_loop(0, n_tiles - 1, pass1, 0)
    for copy in late_copies:
        copy.wait()
    finish_tile(last_tile, False)

    row, col = _iota((gr + 8, 2 * gr), 0), _iota((gr + 8, 2 * gr), 1)
    head = jnp.where(row < gr, (row >= dh).astype(jnp.int32), (row - gr) >> 2)
    own = head == (col & 1)
    for g in range(n_groups):
        read_v[g] = _to_words(jnp.where(own, state_v[g], 0.0))

    def glu(c, hn_ops, hn_rest):
        b = c * FF_CHUNK
        rhs = {j: gate_up_sums_v[c, n] for n, j in enumerate(RHS_SUMS)}
        rhs[1] = jnp.concatenate([w[0:dq, b:b + fh] for w in (wg_v, wu_v)], axis=1)
        rhs[4] = jnp.concatenate([w[dq:2 * dq, b + fh:b + FF_CHUNK] for w in (wg_v, wu_v)], axis=1)
        gate_rest = _dot(hn_rest, wg_v[2 * dq:D, b:b + FF_CHUNK])
        up_rest = _dot(hn_rest, wu_v[2 * dq:D, b:b + FF_CHUNK])
        acts = []
        for n, quad in enumerate(_strassen_out([_dot(hn_ops[j], rhs[j]) for j in range(7)])):
            rows, cols = slice(n // 2 * th, (n // 2 + 1) * th), slice(n % 2 * fh, (n % 2 + 1) * fh)
            acts.append(_gelu(quad[:, 0:fh] + gate_rest[rows, cols]) * (quad[:, fh:FF_CHUNK] + up_rest[rows, cols]))
        act = jnp.concatenate([jnp.concatenate(acts[0:2], axis=1), jnp.concatenate(acts[2:4], axis=1)], axis=0)
        return [a.astype(BF16) for a in _strassen_lhs(*acts) + [act]]

    def down(c, act_ops, acc):
        b = c * FF_CHUNK
        rhs = {j: down_sums_v[c, n] for n, j in enumerate(RHS_SUMS)}
        rhs[1] = wd_v[b:b + fh, 0:dq]
        rhs[4] = wd_v[b + fh:b + FF_CHUNK, dq:2 * dq]
        rhs[7] = wd_v[b:b + FF_CHUNK, 2 * dq:D]
        m = {j: _dot(act_ops[j], rhs[j]) for j in (7, 2, 4, 3, 0, 6, 1, 5)}
        return [m[j] if acc is None else acc[j] + m[j] for j in range(8)]

    def pass2(i, carry):
        first_head = _iota((8, T), 0) < 4
        parts = []
        for g in range(n_groups):
            num_den = _dot(_from_words(read_v[g]), load_phi(i, g))
            both = 1.0 / (num_den[gr:gr + 8] + 1e-6)
            swapped = pltpu.roll(both, 4, 0)
            inv0 = jnp.where(first_head, both, swapped)
            inv1 = jnp.where(first_head, swapped, both)
            parts.append(num_den[0:gr] * jnp.concatenate([inv0, inv0, both, inv1, inv1], axis=0))
        o = jnp.concatenate(parts, axis=0).astype(BF16).T

        hs, hns = [], []
        for r in range(0, T, WO_ROWS):
            hs.append(x_v[i, r:r + WO_ROWS, :].astype(F32) + _dot(o[r:r + WO_ROWS], wo_v[...]))
            hns.append(_layernorm(hs[-1]))
        h = jnp.concatenate(hs, axis=0)
        hn = jnp.concatenate(hns, axis=0)
        hn_ops = [a.astype(BF16) for a in _strassen_lhs(
            hn[0:th, 0:dq], hn[0:th, dq:2 * dq], hn[th:T, 0:dq], hn[th:T, dq:2 * dq])]
        hn_rest = hn[:, 2 * dq:D].astype(BF16)

        acc = None
        act_ops = glu(0, hn_ops, hn_rest)
        for c in range(1, n_chunks):
            nxt = glu(c, hn_ops, hn_rest)
            acc = down(c - 1, act_ops, acc)
            act_ops = nxt
        acc = down(n_chunks - 1, act_ops, acc)
        y11, y12, y21, y22 = _strassen_out(acc[0:7])
        y = h + jnp.concatenate([jnp.concatenate([y11, y12, acc[7][0:th]], axis=1),
                                 jnp.concatenate([y21, y22, acc[7][th:T]], axis=1)], axis=0)
        for u in range(n_out):
            out_v[i * n_out + u] = y[u * OUT_ROWS:(u + 1) * OUT_ROWS].astype(BF16)
            out_copy(i * n_out + u).start()
        return carry

    lax.fori_loop(0, n_tiles, pass2, 0)
    for j in range(n_tiles * n_out):
        out_copy(j).wait()


def build(interpret=False):
    def fn(A_x, A_wqkv, A_w_phi, A_wo, B_x, B_w_gate, B_w_up, B_w_down):
        del B_x
        B, S, D = A_x.shape
        F = B_w_gate.shape[1]
        dh = D // HEADS
        gr = PAIR * dh
        n_tiles = S // TILE
        assert B == 1 and dh == 20 and S % TILE == 0 and n_tiles >= 2 and F % FF_CHUNK == 0
        hbm = pl.BlockSpec(memory_space=pl.ANY)
        out = pl.pallas_call(
            _kernel,
            out_shape=jax.ShapeDtypeStruct((S, D), A_x.dtype),
            in_specs=[hbm] * 7,
            out_specs=hbm,
            scratch_shapes=[
                pltpu.VMEM((n_tiles, TILE, D), BF16),
                pltpu.VMEM((D, D), BF16),
                pltpu.VMEM((WK_SPLIT, D), BF16),
                pltpu.VMEM((D - WK_SPLIT, D), BF16),
                pltpu.VMEM((D, D), BF16),
                pltpu.VMEM((dh, dh, HEADS), BF16),
                pltpu.VMEM((D, D), BF16),
                pltpu.VMEM((D, F), BF16),
                pltpu.VMEM((D, F), BF16),
                pltpu.VMEM((F, D), BF16),
                pltpu.VMEM((F // FF_CHUNK, 5, 2 * LANES, FF_CHUNK), BF16),
                pltpu.VMEM((F // FF_CHUNK, 5, FF_CHUNK // 2, 2 * LANES), BF16),
                pltpu.VMEM((D // LANES, 2 * gr, LANES), U32),
                pltpu.VMEM((3, D // 2, D), U32),
                pltpu.VMEM((TILE // 2, D), U32),
                pltpu.VMEM((D, TILE), F32),
                pltpu.VMEM((n_tiles + 1, D, TILE), U32),
                pltpu.VMEM((HEADS // PAIR, gr + 8, 2 * gr), F32),
                pltpu.VMEM((HEADS // PAIR, gr // 2 + 4, 2 * gr), U32),
                pltpu.VMEM((S // OUT_ROWS, OUT_ROWS, D), BF16),
                pltpu.SemaphoreType.DMA((n_tiles,)),
                pltpu.SemaphoreType.DMA((10,)),
                pltpu.SemaphoreType.DMA((S // OUT_ROWS,)),
            ],
            compiler_params=pltpu.CompilerParams(vmem_limit_bytes=100 * 1024 * 1024),
            interpret=interpret,
        )(A_x.reshape(S, D), A_wqkv, A_w_phi.transpose(1, 2, 0), A_wo, B_w_gate, B_w_up, B_w_down)
        return out.reshape(B, S, D)
    return fn


pallas_sequential_preLN__linear_kernel_hedgehog__geglu_ffn__prompt_kernel = jax.jit(build())
```

```python
import jax
import jax.numpy as jnp
import numpy as np
from jax import lax
import jax.experimental.pallas as pl
import jax.experimental.pallas.tpu as pltpu

HEADS = 32
PAIR = 2
TILE = 512
WO_ROWS = 64
OUT_ROWS = 128
FF_CHUNK = 256
WK_SPLIT = 384
LANES = 128
LOG2E = float(np.log2(np.e))
GELU_C0 = float(np.sqrt(2.0 / np.pi))
GELU_C1 = GELU_C0 * 0.044715
NT_DIMS = (((1,), (1,)), ((), ()))
F32 = jnp.float32
BF16 = jnp.bfloat16
U32 = jnp.uint32


def _to_words(x):
    return pltpu.bitcast(x.astype(BF16), U32)


def _from_words(x):
    return pltpu.bitcast(x, BF16)


def _dot(a, b):
    return jnp.dot(a, b, preferred_element_type=F32)


def _dot_nt(a, b):
    return lax.dot_general(a, b, NT_DIMS, preferred_element_type=F32)


def _iota(shape, axis):
    return lax.broadcasted_iota(jnp.int32, shape, axis)


def _layernorm(x):
    d = x - jnp.mean(x, axis=-1, keepdims=True)
    return d * lax.rsqrt(jnp.mean(d * d, axis=-1, keepdims=True) + 1e-5)


def _gelu(x):
    return (0.5 * x) * (1.0 + jnp.tanh(x * (GELU_C0 + GELU_C1 * (x * x))))


def _per_head(op, vregs):
    while len(vregs) > 1:
        vregs = [op(*vregs[i:i + 2]) if i + 1 < len(vregs) else vregs[i] for i in range(0, len(vregs), 2)]
    y = vregs[0]
    y = op(y, pltpu.roll(y, 4, 0))
    return op(y, pltpu.roll(y, 2, 0))


def _recip(s):
    r = pl.reciprocal(s, approx=True)
    return r * (2.0 - s * r)


def _feature_map(p):
    rows = [p[j:j + 8] for j in range(0, p.shape[0], 8)]
    hi = _per_head(jnp.maximum, rows)
    lo = _per_head(jnp.minimum, rows)
    pos = [jnp.exp2(r - hi) for r in rows]
    neg = [jnp.exp2(lo - r) for r in rows]
    pos_scale = _recip(_per_head(jnp.add, pos))
    neg_scale = _recip(_per_head(jnp.add, neg))
    return jnp.concatenate([e * pos_scale for e in pos] + [e * neg_scale for e in neg], axis=0)


def _strassen_lhs(a11, a12, a21, a22):
    return [a11 + a22, a21 + a22, a11, a22, a11 + a12, a21 - a11, a12 - a22]


def _strassen_rhs(b11, b12, b21, b22):
    return [b11 + b22, b11, b12 - b22, b21 - b11, b22, b11 + b12, b21 + b22]


def _strassen_out(m):
    return (m[0] + m[3]) + (m[6] - m[4]), m[2] + m[4], m[1] + m[3], (m[0] - m[1]) + (m[2] + m[5])


def _kernel(x_hbm, wqkv_hbm, wphi_hbm, wo_hbm, wg_hbm, wu_hbm, wd_hbm, out_hbm,
            x_v, wq_v, wka_v, wkb_v, wv_v, wphi_v, wo_v, wg_v, wu_v, wd_v,
            band_v, wt_v, xn_v, kt_v, phi_v, state_v, read_v, out_v,
            x_sem, w_sem, out_sem):
    n_tiles, T, D = x_v.shape
    F = wg_v.shape[1]
    dh = D // HEADS
    n_groups = HEADS // PAIR
    gr = PAIR * dh
    n_out = T // OUT_ROWS
    n_chunks = F // FF_CHUNK
    th, dq, fh = T // 2, 2 * LANES, FF_CHUNK // 2
    k_tiles = D // LANES
    Q, K, V = range(3)

    def x_copy(i):
        rows = pl.ds(pl.multiple_of(i * T, T), T)
        return pltpu.make_async_copy(x_hbm.at[rows], x_v.at[i], x_sem.at[i])

    def out_copy(j):
        rows = pl.ds(pl.multiple_of(j * OUT_ROWS, OUT_ROWS), OUT_ROWS)
        return pltpu.make_async_copy(out_v.at[j], out_hbm.at[rows], out_sem.at[j])

    half = T // 2
    first_x_copies = [
        pltpu.make_async_copy(x_hbm.at[pl.ds(lo, half)], x_v.at[0, pl.ds(lo, half)], sem)
        for lo, sem in ((0, x_sem.at[0]), (half, w_sem.at[9]))]
    wq_copy = pltpu.make_async_copy(wqkv_hbm.at[:, pl.ds(Q * D, D)], wq_v, w_sem.at[0])
    wka_copy = pltpu.make_async_copy(wqkv_hbm.at[pl.ds(0, WK_SPLIT), pl.ds(K * D, D)], wka_v, w_sem.at[1])
    wkb_copy = pltpu.make_async_copy(wqkv_hbm.at[pl.ds(WK_SPLIT, D - WK_SPLIT), pl.ds(K * D, D)], wkb_v,
                                     w_sem.at[2])
    wv_copy = pltpu.make_async_copy(wqkv_hbm.at[:, pl.ds(V * D, D)], wv_v, w_sem.at[3])
    wphi_copy = pltpu.make_async_copy(wphi_hbm, wphi_v, w_sem.at[4])
    late_copies = [pltpu.make_async_copy(src, dst, w_sem.at[5 + n]) for n, (src, dst) in enumerate(
        [(wo_hbm, wo_v), (wg_hbm, wg_v), (wu_hbm, wu_v), (wd_hbm, wd_v)])]

    wphi_copy.start()
    wka_copy.start()
    state_v[...] = jnp.zeros(state_v.shape, F32)
    wphi_copy.wait()
    wkb_copy.start()

    flat = jnp.concatenate([wphi_v[d].astype(F32) for d in range(dh)], axis=1)
    flat = jnp.concatenate([flat, jnp.zeros((HEADS - dh, D), F32)], axis=0).astype(BF16)
    src = _iota((D, D), 0)
    swap = jnp.where(_iota((D, D), 1) == (src & (HEADS - 1)) * dh + (src >> 5), 1.0, 0.0).astype(BF16)
    flat = _dot(flat, swap).astype(BF16)
    row, col = _iota((gr, LANES), 0), _iota((gr, LANES), 1)
    repeat = jnp.where((row >> 1) == col, 1.0, 0.0).astype(BF16)[:, 0:HEADS]
    flat = _dot(repeat, flat)
    overlap = [[g for g in range(n_groups) if g * gr < (j + 1) * LANES and (g + 1) * gr > j * LANES]
               for j in range(k_tiles)]
    for copy in first_x_copies:
        copy.start()
    for j in range(k_tiles):
        blocks = []
        for g in overlap[j]:
            first = (PAIR * g + (row & 1)) * dh - j * LANES
            blocks.append(jnp.where((col >= first) & (col < first + dh),
                                    flat[:, j * LANES:(j + 1) * LANES], 0.0))
        band_v[j] = _to_words(jnp.concatenate(blocks, axis=0))

    def fold(which, w_ref, lo):
        acc = [None] * n_groups
        for j in range(k_tiles):
            res = _dot_nt(_from_words(band_v[j]), w_ref[:, j * LANES:(j + 1) * LANES])
            for n, g in enumerate(overlap[j]):
                part = res[n * gr:(n + 1) * gr]
                acc[g] = part if acc[g] is None else acc[g] + part
        wt_v[which, :, lo:lo + w_ref.shape[0]] = _to_words(jnp.concatenate(acc, axis=0) * LOG2E)

    def project(which, xn):
        return _dot_nt(_from_words(wt_v[which]), xn)

    def store_phi(slot, logits):
        for g in range(n_groups):
            phi = _feature_map(logits[g * gr:(g + 1) * gr, :])
            for c in range(0, T, LANES):
                phi_v[slot, g * gr:(g + 1) * gr, c:c + LANES] = _to_words(phi[:, c:c + LANES])

    def load_phi(slot, g):
        return _from_words(phi_v[slot, g * gr:(g + 1) * gr, :])

    def start_tile(i):
        xn = _layernorm(x_v[i].astype(F32)).astype(BF16)
        xn_v[...] = _to_words(xn)
        kt_v[...] = project(K, xn)

    def finish_tile(i, start_next):
        xn = _from_words(xn_v[...])
        qt = project(Q, xn)
        store_phi(n_tiles, kt_v)
        vt = project(V, xn)
        if not start_next:
            store_phi(i, qt)
        ones = jnp.ones((8, T), F32)
        for g in range(n_groups):
            v_ones = jnp.concatenate([vt[g * gr:(g + 1) * gr], ones], axis=0).astype(BF16)
            state_v[g] += _dot_nt(v_ones, load_phi(n_tiles, g))
        if start_next:
            start_tile(i + 1)
            store_phi(i, qt)

    wka_copy.wait()
    fold(K, wka_v, 0)
    wkb_copy.wait()
    wv_copy.start()
    wq_copy.start()
    fold(K, wkb_v, WK_SPLIT)
    for n, copy in enumerate(first_x_copies):
        copy.wait()
        xn = _layernorm(x_v[0, n * half:(n + 1) * half, :].astype(F32))
        xn_v[n * half // 2:(n + 1) * half // 2, :] = _to_words(xn)
    kt_v[...] = project(K, _from_words(xn_v[...]))
    x_copy(1).start()
    wv_copy.wait()
    wq_copy.wait()
    for i in range(2, n_tiles):
        x_copy(i).start()
    for copy in late_copies:
        copy.start()
    wt_v[V] = _to_words(wv_v[...].T)
    fold(Q, wq_v, 0)

    def pass1(i, count):
        x_copy(i + 1).wait()
        finish_tile(i, True)
        return count + 1

    finish_tile(lax.fori_loop(0, n_tiles - 1, pass1, 0), False)

    row, col = _iota((gr + 8, 2 * gr), 0), _iota((gr + 8, 2 * gr), 1)
    head = jnp.where(row < gr, (row >= dh).astype(jnp.int32), (row - gr) >> 2)
    own = head == (col & 1)
    for g in range(n_groups):
        read_v[g] = _to_words(jnp.where(own, state_v[g], 0.0))
    for copy in late_copies:
        copy.wait()

    def weight_operands(w_ref, r0, rn, c0, cn):
        blocks = [w_ref[r0 + a * rn:r0 + (a + 1) * rn, c0 + b * cn:c0 + (b + 1) * cn]
                  for a in range(2) for b in range(2)]
        ops = [w.astype(BF16) for w in _strassen_rhs(*[w.astype(F32) for w in blocks])]
        ops[1], ops[4] = blocks[0], blocks[3]
        return ops

    def glu(c, hn_ops, hn_rest):
        b = c * FF_CHUNK
        rhs = [jnp.concatenate(pair, axis=1) for pair in zip(
            weight_operands(wg_v, 0, dq, b, fh), weight_operands(wu_v, 0, dq, b, fh))]
        gate_rest = _dot(hn_rest, wg_v[2 * dq:D, b:b + FF_CHUNK])
        up_rest = _dot(hn_rest, wu_v[2 * dq:D, b:b + FF_CHUNK])
        acts = []
        for n, quad in enumerate(_strassen_out([_dot(hn_ops[j], rhs[j]) for j in range(7)])):
            rows, cols = slice(n // 2 * th, (n // 2 + 1) * th), slice(n % 2 * fh, (n % 2 + 1) * fh)
            acts.append(_gelu(quad[:, 0:fh] + gate_rest[rows, cols]) * (quad[:, fh:FF_CHUNK] + up_rest[rows, cols]))
        act = jnp.concatenate([jnp.concatenate(acts[0:2], axis=1), jnp.concatenate(acts[2:4], axis=1)], axis=0)
        return [a.astype(BF16) for a in _strassen_lhs(*acts) + [act]]

    def down(c, act_ops, acc):
        b = c * FF_CHUNK
        rhs = weight_operands(wd_v, b, fh, 0, dq) + [wd_v[b:b + FF_CHUNK, 2 * dq:D]]
        m = {j: _dot(act_ops[j], rhs[j]) for j in (7, 2, 4, 3, 0, 6, 1, 5)}
        return [m[j] if acc is None else acc[j] + m[j] for j in range(8)]

    def pass2(i, carry):
        first_head = _iota((8, T), 0) < 4
        parts = []
        for g in range(n_groups):
            num_den = _dot(_from_words(read_v[g]), load_phi(i, g))
            both = 1.0 / (num_den[gr:gr + 8] + 1e-6)
            swapped = pltpu.roll(both, 4, 0)
            inv0 = jnp.where(first_head, both, swapped)
            inv1 = jnp.where(first_head, swapped, both)
            parts.append(num_den[0:gr] * jnp.concatenate([inv0, inv0, both, inv1, inv1], axis=0))
        o = jnp.concatenate(parts, axis=0).astype(BF16).T

        hs, hns = [], []
        for r in range(0, T, WO_ROWS):
            hs.append(x_v[i, r:r + WO_ROWS, :].astype(F32) + _dot(o[r:r + WO_ROWS], wo_v[...]))
            hns.append(_layernorm(hs[-1]))
        h = jnp.concatenate(hs, axis=0)
        hn = jnp.concatenate(hns, axis=0)
        hn_ops = [a.astype(BF16) for a in _strassen_lhs(
            hn[0:th, 0:dq], hn[0:th, dq:2 * dq], hn[th:T, 0:dq], hn[th:T, dq:2 * dq])]
        hn_rest = hn[:, 2 * dq:D].astype(BF16)

        acc = None
        act_ops = glu(0, hn_ops, hn_rest)
        for c in range(1, n_chunks):
            nxt = glu(c, hn_ops, hn_rest)
            acc = down(c - 1, act_ops, acc)
            act_ops = nxt
        acc = down(n_chunks - 1, act_ops, acc)
        y11, y12, y21, y22 = _strassen_out(acc[0:7])
        y = h + jnp.concatenate([jnp.concatenate([y11, y12, acc[7][0:th]], axis=1),
                                 jnp.concatenate([y21, y22, acc[7][th:T]], axis=1)], axis=0)
        for u in range(n_out):
            out_v[i * n_out + u] = y[u * OUT_ROWS:(u + 1) * OUT_ROWS].astype(BF16)
            out_copy(i * n_out + u).start()
        return carry

    lax.fori_loop(0, n_tiles, pass2, 0)
    for j in range(n_tiles * n_out):
        out_copy(j).wait()


def build(interpret=False):
    def fn(A_x, A_wqkv, A_w_phi, A_wo, B_x, B_w_gate, B_w_up, B_w_down):
        del B_x
        B, S, D = A_x.shape
        F = B_w_gate.shape[1]
        dh = D // HEADS
        gr = PAIR * dh
        n_tiles = S // TILE
        assert B == 1 and dh == 20 and S % TILE == 0 and n_tiles >= 2 and F % FF_CHUNK == 0
        hbm = pl.BlockSpec(memory_space=pl.ANY)
        out = pl.pallas_call(
            _kernel,
            out_shape=jax.ShapeDtypeStruct((S, D), A_x.dtype),
            in_specs=[hbm] * 7,
            out_specs=hbm,
            scratch_shapes=[
                pltpu.VMEM((n_tiles, TILE, D), BF16),
                pltpu.VMEM((D, D), BF16),
                pltpu.VMEM((WK_SPLIT, D), BF16),
                pltpu.VMEM((D - WK_SPLIT, D), BF16),
                pltpu.VMEM((D, D), BF16),
                pltpu.VMEM((dh, dh, HEADS), BF16),
                pltpu.VMEM((D, D), BF16),
                pltpu.VMEM((D, F), BF16),
                pltpu.VMEM((D, F), BF16),
                pltpu.VMEM((F, D), BF16),
                pltpu.VMEM((D // LANES, 2 * gr, LANES), U32),
                pltpu.VMEM((3, D // 2, D), U32),
                pltpu.VMEM((TILE // 2, D), U32),
                pltpu.VMEM((D, TILE), F32),
                pltpu.VMEM((n_tiles + 1, D, TILE), U32),
                pltpu.VMEM((HEADS // PAIR, gr + 8, 2 * gr), F32),
                pltpu.VMEM((HEADS // PAIR, gr // 2 + 4, 2 * gr), U32),
                pltpu.VMEM((S // OUT_ROWS, OUT_ROWS, D), BF16),
                pltpu.SemaphoreType.DMA((n_tiles,)),
                pltpu.SemaphoreType.DMA((10,)),
                pltpu.SemaphoreType.DMA((S // OUT_ROWS,)),
            ],
            compiler_params=pltpu.CompilerParams(vmem_limit_bytes=100 * 1024 * 1024),
            interpret=interpret,
        )(A_x.reshape(S, D), A_wqkv, A_w_phi.transpose(1, 2, 0), A_wo, B_w_gate, B_w_up, B_w_down)
        return out.reshape(B, S, D)
    return fn


pallas_sequential_preLN__linear_kernel_hedgehog__geglu_ffn__prompt_kernel = jax.jit(build())
```

```python
import jax
import jax.numpy as jnp
import numpy as np
from jax import lax
import jax.experimental.pallas as pl
import jax.experimental.pallas.tpu as pltpu

HEADS = 32
PAIR = 2
TILE = 512
WO_ROWS = 64
OUT_ROWS = 128
FF_CHUNK = 256
WK_SPLIT = 384
LANES = 128
LOG2E = float(np.log2(np.e))
GELU_C0 = float(np.sqrt(2.0 / np.pi))
GELU_C1 = GELU_C0 * 0.044715
NT_DIMS = (((1,), (1,)), ((), ()))
F32 = jnp.float32
BF16 = jnp.bfloat16
U32 = jnp.uint32


def _to_words(x):
    return pltpu.bitcast(x.astype(BF16), U32)


def _from_words(x):
    return pltpu.bitcast(x, BF16)


def _dot(a, b):
    return jnp.dot(a, b, preferred_element_type=F32)


def _dot_nt(a, b):
    return lax.dot_general(a, b, NT_DIMS, preferred_element_type=F32)


def _iota(shape, axis):
    return lax.broadcasted_iota(jnp.int32, shape, axis)


def _layernorm(x):
    d = x - jnp.mean(x, axis=-1, keepdims=True)
    return d * lax.rsqrt(jnp.mean(d * d, axis=-1, keepdims=True) + 1e-5)


def _gelu(x):
    return (0.5 * x) * (1.0 + jnp.tanh(x * (GELU_C0 + GELU_C1 * (x * x))))


def _per_head(op, vregs):
    while len(vregs) > 1:
        vregs = [op(*vregs[i:i + 2]) if i + 1 < len(vregs) else vregs[i] for i in range(0, len(vregs), 2)]
    y = vregs[0]
    y = op(y, pltpu.roll(y, 4, 0))
    return op(y, pltpu.roll(y, 2, 0))


def _recip(s):
    r = pl.reciprocal(s, approx=True)
    return r * (2.0 - s * r)


def _feature_map(p):
    rows = [p[j:j + 8] for j in range(0, p.shape[0], 8)]
    hi = _per_head(jnp.maximum, rows)
    lo = _per_head(jnp.minimum, rows)
    pos = [jnp.exp2(r - hi) for r in rows]
    neg = [jnp.exp2(lo - r) for r in rows]
    pos_scale = _recip(_per_head(jnp.add, pos))
    neg_scale = _recip(_per_head(jnp.add, neg))
    return jnp.concatenate([e * pos_scale for e in pos] + [e * neg_scale for e in neg], axis=0)


def _strassen_lhs(a11, a12, a21, a22):
    return [a11 + a22, a21 + a22, a11, a22, a11 + a12, a21 - a11, a12 - a22]


def _strassen_rhs_bf16(b11, b12, b21, b22):
    f11, f12, f21, f22 = [b.astype(F32) for b in (b11, b12, b21, b22)]
    return [b.astype(BF16) for b in (f11 + f22, b11, f12 - f22, f21 - f11, b22, f11 + f12, f21 + f22)]


def _strassen_out(m):
    return (m[0] + m[3]) + (m[6] - m[4]), m[2] + m[4], m[1] + m[3], (m[0] - m[1]) + (m[2] + m[5])


def _kernel(x_hbm, wqkv_hbm, wphi_hbm, wo_hbm, wg_hbm, wu_hbm, wd_hbm, out_hbm,
            x_v, wq_v, wka_v, wkb_v, wv_v, wphi_v, wo_v, wg_v, wu_v, wd_v,
            band_v, wt_v, wv_ops_v, wv_rest_v, xn_v, kt_v, phi_v, state_v, read_v, out_v,
            x_sem, w_sem, out_sem):
    n_tiles, T, D = x_v.shape
    F = wg_v.shape[1]
    dh = D // HEADS
    n_groups = HEADS // PAIR
    gr = PAIR * dh
    n_out = T // OUT_ROWS
    n_chunks = F // FF_CHUNK
    th, dq, fh = T // 2, 2 * LANES, FF_CHUNK // 2
    k_tiles = D // LANES
    Q, K, V = range(3)

    def x_copy(i):
        rows = pl.ds(pl.multiple_of(i * T, T), T)
        return pltpu.make_async_copy(x_hbm.at[rows], x_v.at[i], x_sem.at[i])

    def out_copy(j):
        rows = pl.ds(pl.multiple_of(j * OUT_ROWS, OUT_ROWS), OUT_ROWS)
        return pltpu.make_async_copy(out_v.at[j], out_hbm.at[rows], out_sem.at[j])

    half = T // 2
    first_x_copies = [
        pltpu.make_async_copy(x_hbm.at[pl.ds(lo, half)], x_v.at[0, pl.ds(lo, half)], sem)
        for lo, sem in ((0, x_sem.at[0]), (half, w_sem.at[9]))]
    wq_copy = pltpu.make_async_copy(wqkv_hbm.at[:, pl.ds(Q * D, D)], wq_v, w_sem.at[0])
    wka_copy = pltpu.make_async_copy(wqkv_hbm.at[pl.ds(0, WK_SPLIT), pl.ds(K * D, D)], wka_v, w_sem.at[1])
    wkb_copy = pltpu.make_async_copy(wqkv_hbm.at[pl.ds(WK_SPLIT, D - WK_SPLIT), pl.ds(K * D, D)], wkb_v,
                                     w_sem.at[2])
    wv_copy = pltpu.make_async_copy(wqkv_hbm.at[:, pl.ds(V * D, D)], wv_v, w_sem.at[3])
    wphi_copy = pltpu.make_async_copy(wphi_hbm, wphi_v, w_sem.at[4])
    late_copies = [pltpu.make_async_copy(src, dst, w_sem.at[5 + n]) for n, (src, dst) in enumerate(
        [(wo_hbm, wo_v), (wg_hbm, wg_v), (wu_hbm, wu_v), (wd_hbm, wd_v)])]

    wphi_copy.start()
    wka_copy.start()
    state_v[...] = jnp.zeros(state_v.shape, F32)
    wphi_copy.wait()
    wkb_copy.start()

    flat = jnp.concatenate([wphi_v[d].astype(F32) for d in range(dh)], axis=1)
    flat = jnp.concatenate([flat, jnp.zeros((HEADS - dh, D), F32)], axis=0).astype(BF16)
    src = _iota((D, D), 0)
    swap = jnp.where(_iota((D, D), 1) == (src & (HEADS - 1)) * dh + (src >> 5), 1.0, 0.0).astype(BF16)
    flat = _dot(flat, swap).astype(BF16)
    row, col = _iota((gr, LANES), 0), _iota((gr, LANES), 1)
    repeat = jnp.where((row >> 1) == col, 1.0, 0.0).astype(BF16)[:, 0:HEADS]
    flat = _dot(repeat, flat)
    overlap = [[g for g in range(n_groups) if g * gr < (j + 1) * LANES and (g + 1) * gr > j * LANES]
               for j in range(k_tiles)]
    for copy in first_x_copies:
        copy.start()
    for j in range(k_tiles):
        blocks = []
        for g in overlap[j]:
            first = (PAIR * g + (row & 1)) * dh - j * LANES
            blocks.append(jnp.where((col >= first) & (col < first + dh),
                                    flat[:, j * LANES:(j + 1) * LANES], 0.0))
        band_v[j] = _to_words(jnp.concatenate(blocks, axis=0))

    def fold(which, w_ref, lo):
        acc = [None] * n_groups
        for j in range(k_tiles):
            res = _dot_nt(_from_words(band_v[j]), w_ref[:, j * LANES:(j + 1) * LANES])
            for n, g in enumerate(overlap[j]):
                part = res[n * gr:(n + 1) * gr]
                acc[g] = part if acc[g] is None else acc[g] + part
        wt_v[which, :, lo:lo + w_ref.shape[0]] = _to_words(jnp.concatenate(acc, axis=0) * LOG2E)

    def project(which, xn):
        return _dot_nt(_from_words(wt_v[which]), xn)

    def project_v(xn):
        ops = _strassen_rhs_bf16(xn[0:th, 0:dq], xn[th:T, 0:dq], xn[0:th, dq:2 * dq], xn[th:T, dq:2 * dq])
        rest = _dot_nt(_from_words(wv_rest_v[...]), xn[:, 2 * dq:D])
        c11, c12, c21, c22 = _strassen_out([_dot_nt(_from_words(wv_ops_v[j]), ops[j]) for j in range(7)])
        return rest + jnp.concatenate(
            [jnp.concatenate([c11, c12], axis=1), jnp.concatenate([c21, c22], axis=1)], axis=0)

    def store_phi(slot, logits):
        for g in range(n_groups):
            phi = _feature_map(logits[g * gr:(g + 1) * gr, :])
            for c in range(0, T, LANES):
                phi_v[slot, g * gr:(g + 1) * gr, c:c + LANES] = _to_words(phi[:, c:c + LANES])

    def load_phi(slot, g):
        return _from_words(phi_v[slot, g * gr:(g + 1) * gr, :])

    def start_tile(i):
        xn = _layernorm(x_v[i].astype(F32)).astype(BF16)
        xn_v[...] = _to_words(xn)
        kt_v[...] = project(K, xn)

    def finish_tile(i, start_next):
        xn = _from_words(xn_v[...])
        qt = project(Q, xn)
        store_phi(n_tiles, kt_v)
        vt = project_v(xn)
        if not start_next:
            store_phi(i, qt)
        ones = jnp.ones((8, T), F32)
        for g in range(n_groups):
            v_ones = jnp.concatenate([vt[g * gr:(g + 1) * gr], ones], axis=0).astype(BF16)
            state_v[g] += _dot_nt(v_ones, load_phi(n_tiles, g))
        if start_next:
            start_tile(i + 1)
            store_phi(i, qt)

    wka_copy.wait()
    fold(K, wka_v, 0)
    wkb_copy.wait()
    wv_copy.start()
    wq_copy.start()
    fold(K, wkb_v, WK_SPLIT)
    for n, copy in enumerate(first_x_copies):
        copy.wait()
        xn = _layernorm(x_v[0, n * half:(n + 1) * half, :].astype(F32))
        xn_v[n * half // 2:(n + 1) * half // 2, :] = _to_words(xn)
    kt_v[...] = project(K, _from_words(xn_v[...]))
    x_copy(1).start()
    wv_copy.wait()
    wq_copy.wait()
    for i in range(2, n_tiles):
        x_copy(i).start()
    for copy in late_copies:
        copy.start()
    wvt = wv_v[...].T.astype(F32)
    for j, block in enumerate(_strassen_lhs(wvt[0:D // 2, 0:dq], wvt[0:D // 2, dq:2 * dq],
                                            wvt[D // 2:D, 0:dq], wvt[D // 2:D, dq:2 * dq])):
        wv_ops_v[j] = _to_words(block)
    wv_rest_v[...] = _to_words(wvt[:, 2 * dq:D])
    fold(Q, wq_v, 0)

    def pass1(i, count):
        x_copy(i + 1).wait()
        finish_tile(i, True)
        return count + 1

    finish_tile(lax.fori_loop(0, n_tiles - 1, pass1, 0), False)

    row, col = _iota((gr + 8, 2 * gr), 0), _iota((gr + 8, 2 * gr), 1)
    head = jnp.where(row < gr, (row >= dh).astype(jnp.int32), (row - gr) >> 2)
    own = head == (col & 1)
    for g in range(n_groups):
        read_v[g] = _to_words(jnp.where(own, state_v[g], 0.0))
    for copy in late_copies:
        copy.wait()

    def weight_operands(w_ref, r0, rn, c0, cn):
        return _strassen_rhs_bf16(*[w_ref[r0 + a * rn:r0 + (a + 1) * rn, c0 + b * cn:c0 + (b + 1) * cn]
                                    for a in range(2) for b in range(2)])

    def glu(c, hn_ops, hn_rest):
        b = c * FF_CHUNK
        rhs = [jnp.concatenate(pair, axis=1) for pair in zip(
            weight_operands(wg_v, 0, dq, b, fh), weight_operands(wu_v, 0, dq, b, fh))]
        gate_rest = _dot(hn_rest, wg_v[2 * dq:D, b:b + FF_CHUNK])
        up_rest = _dot(hn_rest, wu_v[2 * dq:D, b:b + FF_CHUNK])
        acts = []
        for n, quad in enumerate(_strassen_out([_dot(hn_ops[j], rhs[j]) for j in range(7)])):
            rows, cols = slice(n // 2 * th, (n // 2 + 1) * th), slice(n % 2 * fh, (n % 2 + 1) * fh)
            acts.append(_gelu(quad[:, 0:fh] + gate_rest[rows, cols]) * (quad[:, fh:FF_CHUNK] + up_rest[rows, cols]))
        act = jnp.concatenate([jnp.concatenate(acts[0:2], axis=1), jnp.concatenate(acts[2:4], axis=1)], axis=0)
        return [a.astype(BF16) for a in _strassen_lhs(*acts) + [act]]

    def down(c, act_ops, acc):
        b = c * FF_CHUNK
        rhs = weight_operands(wd_v, b, fh, 0, dq) + [wd_v[b:b + FF_CHUNK, 2 * dq:D]]
        m = {j: _dot(act_ops[j], rhs[j]) for j in (7, 2, 4, 3, 0, 6, 1, 5)}
        return [m[j] if acc is None else acc[j] + m[j] for j in range(8)]

    def pass2(i, carry):
        first_head = _iota((8, T), 0) < 4
        parts = []
        for g in range(n_groups):
            num_den = _dot(_from_words(read_v[g]), load_phi(i, g))
            both = 1.0 / (num_den[gr:gr + 8] + 1e-6)
            swapped = pltpu.roll(both, 4, 0)
            inv0 = jnp.where(first_head, both, swapped)
            inv1 = jnp.where(first_head, swapped, both)
            parts.append(num_den[0:gr] * jnp.concatenate([inv0, inv0, both, inv1, inv1], axis=0))
        o = jnp.concatenate(parts, axis=0).astype(BF16).T

        hs, hns = [], []
        for r in range(0, T, WO_ROWS):
            hs.append(x_v[i, r:r + WO_ROWS, :].astype(F32) + _dot(o[r:r + WO_ROWS], wo_v[...]))
            hns.append(_layernorm(hs[-1]))
        h = jnp.concatenate(hs, axis=0)
        hn = jnp.concatenate(hns, axis=0)
        hn_ops = [a.astype(BF16) for a in _strassen_lhs(
            hn[0:th, 0:dq], hn[0:th, dq:2 * dq], hn[th:T, 0:dq], hn[th:T, dq:2 * dq])]
        hn_rest = hn[:, 2 * dq:D].astype(BF16)

        acc = None
        act_ops = glu(0, hn_ops, hn_rest)
        for c in range(1, n_chunks):
            nxt = glu(c, hn_ops, hn_rest)
            acc = down(c - 1, act_ops, acc)
            act_ops = nxt
        acc = down(n_chunks - 1, act_ops, acc)
        y11, y12, y21, y22 = _strassen_out(acc[0:7])
        y = h + jnp.concatenate([jnp.concatenate([y11, y12, acc[7][0:th]], axis=1),
                                 jnp.concatenate([y21, y22, acc[7][th:T]], axis=1)], axis=0)
        for u in range(n_out):
            out_v[i * n_out + u] = y[u * OUT_ROWS:(u + 1) * OUT_ROWS].astype(BF16)
            out_copy(i * n_out + u).start()
        return carry

    lax.fori_loop(0, n_tiles, pass2, 0)
    for j in range(n_tiles * n_out):
        out_copy(j).wait()


def build(interpret=False):
    def fn(A_x, A_wqkv, A_w_phi, A_wo, B_x, B_w_gate, B_w_up, B_w_down):
        del B_x
        B, S, D = A_x.shape
        F = B_w_gate.shape[1]
        dh = D // HEADS
        gr = PAIR * dh
        n_tiles = S // TILE
        assert B == 1 and D == 5 * LANES and S % TILE == 0 and n_tiles >= 2 and F % FF_CHUNK == 0
        hbm = pl.BlockSpec(memory_space=pl.ANY)
        out = pl.pallas_call(
            _kernel,
            out_shape=jax.ShapeDtypeStruct((S, D), A_x.dtype),
            in_specs=[hbm] * 7,
            out_specs=hbm,
            scratch_shapes=[
                pltpu.VMEM((n_tiles, TILE, D), BF16),
                pltpu.VMEM((D, D), BF16),
                pltpu.VMEM((WK_SPLIT, D), BF16),
                pltpu.VMEM((D - WK_SPLIT, D), BF16),
                pltpu.VMEM((D, D), BF16),
                pltpu.VMEM((dh, dh, HEADS), BF16),
                pltpu.VMEM((D, D), BF16),
                pltpu.VMEM((D, F), BF16),
                pltpu.VMEM((D, F), BF16),
                pltpu.VMEM((F, D), BF16),
                pltpu.VMEM((D // LANES, 2 * gr, LANES), U32),
                pltpu.VMEM((2, D // 2, D), U32),
                pltpu.VMEM((7, D // 4, 2 * LANES), U32),
                pltpu.VMEM((D // 2, D - 4 * LANES), U32),
                pltpu.VMEM((TILE // 2, D), U32),
                pltpu.VMEM((D, TILE), F32),
                pltpu.VMEM((n_tiles + 1, D, TILE), U32),
                pltpu.VMEM((HEADS // PAIR, gr + 8, 2 * gr), F32),
                pltpu.VMEM((HEADS // PAIR, gr // 2 + 4, 2 * gr), U32),
                pltpu.VMEM((S // OUT_ROWS, OUT_ROWS, D), BF16),
                pltpu.SemaphoreType.DMA((n_tiles,)),
                pltpu.SemaphoreType.DMA((10,)),
                pltpu.SemaphoreType.DMA((S // OUT_ROWS,)),
            ],
            compiler_params=pltpu.CompilerParams(vmem_limit_bytes=100 * 1024 * 1024),
            interpret=interpret,
        )(A_x.reshape(S, D), A_wqkv, A_w_phi.transpose(1, 2, 0), A_wo, B_w_gate, B_w_up, B_w_down)
        return out.reshape(B, S, D)
    return fn


pallas_sequential_preLN__linear_kernel_hedgehog__geglu_ffn__prompt_kernel = jax.jit(build())
```

```python
import jax
import jax.numpy as jnp
import numpy as np
from jax import lax
import jax.experimental.pallas as pl
import jax.experimental.pallas.tpu as pltpu

HEADS = 32
PAIR = 2
TILE = 512
WO_ROWS = 64
OUT_ROWS = 128
FF_CHUNK = 256
WK_SPLIT = 384
LANES = 128
LOG2E = float(np.log2(np.e))
GELU_C0 = float(np.sqrt(2.0 / np.pi))
GELU_C1 = GELU_C0 * 0.044715
NT_DIMS = (((1,), (1,)), ((), ()))
F32 = jnp.float32
BF16 = jnp.bfloat16
U32 = jnp.uint32


def _to_words(x):
    return pltpu.bitcast(x.astype(BF16), U32)


def _from_words(x):
    return pltpu.bitcast(x, BF16)


def _dot(a, b):
    return jnp.dot(a, b, preferred_element_type=F32)


def _dot_nt(a, b):
    return lax.dot_general(a, b, NT_DIMS, preferred_element_type=F32)


def _iota(shape, axis):
    return lax.broadcasted_iota(jnp.int32, shape, axis)


def _layernorm(x):
    d = x - jnp.mean(x, axis=-1, keepdims=True)
    return d * lax.rsqrt(jnp.mean(d * d, axis=-1, keepdims=True) + 1e-5)


def _gelu(x):
    return (0.5 * x) * (1.0 + jnp.tanh(x * (GELU_C0 + GELU_C1 * (x * x))))


def _per_head(op, vregs):
    while len(vregs) > 1:
        vregs = [op(*vregs[i:i + 2]) if i + 1 < len(vregs) else vregs[i] for i in range(0, len(vregs), 2)]
    y = vregs[0]
    y = op(y, pltpu.roll(y, 4, 0))
    return op(y, pltpu.roll(y, 2, 0))


def _recip(s):
    r = pl.reciprocal(s, approx=True)
    return r * (2.0 - s * r)


def _feature_map(p):
    rows = [p[j:j + 8] for j in range(0, p.shape[0], 8)]
    hi = _per_head(jnp.maximum, rows)
    lo = _per_head(jnp.minimum, rows)
    pos = [jnp.exp2(r - hi) for r in rows]
    neg = [jnp.exp2(lo - r) for r in rows]
    pos_scale = _recip(_per_head(jnp.add, pos))
    neg_scale = _recip(_per_head(jnp.add, neg))
    return jnp.concatenate([e * pos_scale for e in pos] + [e * neg_scale for e in neg], axis=0)


def _strassen_lhs(a11, a12, a21, a22):
    return [a11 + a22, a21 + a22, a11, a22, a11 + a12, a21 - a11, a12 - a22]


def _strassen_rhs_bf16(b11, b12, b21, b22):
    f11, f12, f21, f22 = [b.astype(F32) for b in (b11, b12, b21, b22)]
    return [b.astype(BF16) for b in (f11 + f22, b11, f12 - f22, f21 - f11, b22, f11 + f12, f21 + f22)]


def _strassen_out(m):
    return (m[0] + m[3]) + (m[6] - m[4]), m[2] + m[4], m[1] + m[3], (m[0] - m[1]) + (m[2] + m[5])


def _kernel(x_hbm, wqkv_hbm, wphi_hbm, wo_hbm, wg_hbm, wu_hbm, wd_hbm, out_hbm,
            x_v, wq_v, wka_v, wkb_v, wv_v, wphi_v, wo_v, wg_v, wu_v, wd_v,
            band_v, wt_v, wv_ops_v, wv_rest_v, xn_v, kt_v, phi_v, state_v, read_v, out_v,
            x_sem, w_sem, out_sem):
    n_tiles, T, D = x_v.shape
    F = wg_v.shape[1]
    dh = D // HEADS
    n_groups = HEADS // PAIR
    gr = PAIR * dh
    n_out = T // OUT_ROWS
    n_chunks = F // FF_CHUNK
    th, dq, fh = T // 2, 2 * LANES, FF_CHUNK // 2
    k_tiles = D // LANES
    Q, K, V = range(3)

    def x_copy(i):
        rows = pl.ds(pl.multiple_of(i * T, T), T)
        return pltpu.make_async_copy(x_hbm.at[rows], x_v.at[i], x_sem.at[i])

    def out_copy(j):
        rows = pl.ds(pl.multiple_of(j * OUT_ROWS, OUT_ROWS), OUT_ROWS)
        return pltpu.make_async_copy(out_v.at[j], out_hbm.at[rows], out_sem.at[j])

    half = T // 2
    first_x_copies = [
        pltpu.make_async_copy(x_hbm.at[pl.ds(lo, half)], x_v.at[0, pl.ds(lo, half)], sem)
        for lo, sem in ((0, x_sem.at[0]), (half, w_sem.at[9]))]
    wq_copy = pltpu.make_async_copy(wqkv_hbm.at[:, pl.ds(Q * D, D)], wq_v, w_sem.at[0])
    wka_copy = pltpu.make_async_copy(wqkv_hbm.at[pl.ds(0, WK_SPLIT), pl.ds(K * D, D)], wka_v, w_sem.at[1])
    wkb_copy = pltpu.make_async_copy(wqkv_hbm.at[pl.ds(WK_SPLIT, D - WK_SPLIT), pl.ds(K * D, D)], wkb_v,
                                     w_sem.at[2])
    wv_copy = pltpu.make_async_copy(wqkv_hbm.at[:, pl.ds(V * D, D)], wv_v, w_sem.at[3])
    wphi_copy = pltpu.make_async_copy(wphi_hbm, wphi_v, w_sem.at[4])
    late_copies = [pltpu.make_async_copy(src, dst, w_sem.at[5 + n]) for n, (src, dst) in enumerate(
        [(wo_hbm, wo_v), (wg_hbm, wg_v), (wu_hbm, wu_v), (wd_hbm, wd_v)])]

    wphi_copy.start()
    wka_copy.start()
    state_v[...] = jnp.zeros(state_v.shape, F32)
    wphi_copy.wait()
    wkb_copy.start()

    flat = jnp.concatenate([wphi_v[d].astype(F32) for d in range(dh)], axis=1)
    flat = jnp.concatenate([flat, jnp.zeros((HEADS - dh, D), F32)], axis=0).astype(BF16)
    src = _iota((D, D), 0)
    swap = jnp.where(_iota((D, D), 1) == (src & (HEADS - 1)) * dh + (src >> 5), 1.0, 0.0).astype(BF16)
    flat = _dot(flat, swap).astype(BF16)
    row, col = _iota((gr, LANES), 0), _iota((gr, LANES), 1)
    repeat = jnp.where((row >> 1) == col, 1.0, 0.0).astype(BF16)[:, 0:HEADS]
    flat = _dot(repeat, flat)
    overlap = [[g for g in range(n_groups) if g * gr < (j + 1) * LANES and (g + 1) * gr > j * LANES]
               for j in range(k_tiles)]
    for copy in first_x_copies:
        copy.start()
    for j in range(k_tiles):
        blocks = []
        for g in overlap[j]:
            first = (PAIR * g + (row & 1)) * dh - j * LANES
            blocks.append(jnp.where((col >= first) & (col < first + dh),
                                    flat[:, j * LANES:(j + 1) * LANES], 0.0))
        band_v[j] = _to_words(jnp.concatenate(blocks, axis=0))

    def fold(which, w_ref, lo):
        acc = [None] * n_groups
        for j in range(k_tiles):
            res = _dot_nt(_from_words(band_v[j]), w_ref[:, j * LANES:(j + 1) * LANES])
            for n, g in enumerate(overlap[j]):
                part = res[n * gr:(n + 1) * gr]
                acc[g] = part if acc[g] is None else acc[g] + part
        wt_v[which, :, lo:lo + w_ref.shape[0]] = _to_words(jnp.concatenate(acc, axis=0) * LOG2E)

    def project(which, xn):
        return _dot_nt(_from_words(wt_v[which]), xn)

    def project_v(xn):
        ops = _strassen_rhs_bf16(xn[0:th, 0:dq], xn[th:T, 0:dq], xn[0:th, dq:2 * dq], xn[th:T, dq:2 * dq])
        rest = _dot_nt(_from_words(wv_rest_v[...]), xn[:, 2 * dq:D])
        c11, c12, c21, c22 = _strassen_out([_dot_nt(_from_words(wv_ops_v[j]), ops[j]) for j in range(7)])
        return rest + jnp.concatenate(
            [jnp.concatenate([c11, c12], axis=1), jnp.concatenate([c21, c22], axis=1)], axis=0)

    def store_phi(slot, logits):
        for g in range(n_groups):
            phi = _feature_map(logits[g * gr:(g + 1) * gr, :])
            for c in range(0, T, LANES):
                phi_v[slot, g * gr:(g + 1) * gr, c:c + LANES] = _to_words(phi[:, c:c + LANES])

    def start_tile(i):
        xn = _layernorm(x_v[i].astype(F32)).astype(BF16)
        xn_v[...] = _to_words(xn)
        kt_v[...] = project(K, xn)

    def finish_tile(i, start_next):
        xn = _from_words(xn_v[...])
        qt = project(Q, xn)
        store_phi(n_tiles, kt_v)
        vt = project_v(xn)
        if not start_next:
            store_phi(i, qt)
        ones = jnp.ones((8, T), F32)
        for g in range(n_groups):
            v_ones = jnp.concatenate([vt[g * gr:(g + 1) * gr], ones], axis=0).astype(BF16)
            state_v[g] += _dot_nt(v_ones, _from_words(phi_v[n_tiles, g * gr:(g + 1) * gr, :]))
        if start_next:
            start_tile(i + 1)
            store_phi(i, qt)

    wka_copy.wait()
    fold(K, wka_v, 0)
    wkb_copy.wait()
    wv_copy.start()
    wq_copy.start()
    fold(K, wkb_v, WK_SPLIT)
    for n, copy in enumerate(first_x_copies):
        copy.wait()
        xn = _layernorm(x_v[0, n * half:(n + 1) * half, :].astype(F32))
        xn_v[n * half // 2:(n + 1) * half // 2, :] = _to_words(xn)
    kt_v[...] = project(K, _from_words(xn_v[...]))
    x_copy(1).start()
    wv_copy.wait()
    wq_copy.wait()
    for i in range(2, n_tiles):
        x_copy(i).start()
    for copy in late_copies:
        copy.start()
    wvt = wv_v[...].T.astype(F32)
    for j, block in enumerate(_strassen_lhs(wvt[0:D // 2, 0:dq], wvt[0:D // 2, dq:2 * dq],
                                            wvt[D // 2:D, 0:dq], wvt[D // 2:D, dq:2 * dq])):
        wv_ops_v[j] = _to_words(block)
    wv_rest_v[...] = _to_words(wvt[:, 2 * dq:D])
    fold(Q, wq_v, 0)

    def pass1(i, count):
        x_copy(i + 1).wait()
        finish_tile(i, True)
        return count + 1

    finish_tile(lax.fori_loop(0, n_tiles - 1, pass1, 0), False)

    row, col = _iota((gr + 8, 2 * gr), 0), _iota((gr + 8, 2 * gr), 1)
    head = jnp.where(row < gr, (row >= dh).astype(jnp.int32), (row - gr) >> 2)
    own = head == (col & 1)
    for g in range(n_groups):
        read_v[g] = _to_words(jnp.where(own, state_v[g], 0.0))
    for copy in late_copies:
        copy.wait()

    def weight_operands(w_ref, r0, rn, c0, cn):
        return _strassen_rhs_bf16(*[w_ref[r0 + a * rn:r0 + (a + 1) * rn, c0 + b * cn:c0 + (b + 1) * cn]
                                    for a in range(2) for b in range(2)])

    def glu(c, hn_ops, hn_rest):
        b = c * FF_CHUNK
        rhs = [jnp.concatenate(pair, axis=1) for pair in zip(
            weight_operands(wg_v, 0, dq, b, fh), weight_operands(wu_v, 0, dq, b, fh))]
        gate_rest = _dot(hn_rest, wg_v[2 * dq:D, b:b + FF_CHUNK])
        up_rest = _dot(hn_rest, wu_v[2 * dq:D, b:b + FF_CHUNK])
        acts = []
        for n, quad in enumerate(_strassen_out([_dot(hn_ops[j], rhs[j]) for j in range(7)])):
            rows, cols = slice(n // 2 * th, (n // 2 + 1) * th), slice(n % 2 * fh, (n % 2 + 1) * fh)
            acts.append(_gelu(quad[:, 0:fh] + gate_rest[rows, cols]) * (quad[:, fh:FF_CHUNK] + up_rest[rows, cols]))
        act = jnp.concatenate([jnp.concatenate(acts[0:2], axis=1), jnp.concatenate(acts[2:4], axis=1)], axis=0)
        return [a.astype(BF16) for a in _strassen_lhs(*acts) + [act]]

    def down(c, act_ops, acc):
        b = c * FF_CHUNK
        rhs = weight_operands(wd_v, b, fh, 0, dq) + [wd_v[b:b + FF_CHUNK, 2 * dq:D]]
        m = {j: _dot(act_ops[j], rhs[j]) for j in (7, 2, 4, 3, 0, 6, 1, 5)}
        return [m[j] if acc is None else acc[j] + m[j] for j in range(8)]

    def pass2(i, carry):
        first_head = _iota((8, th), 0) < 4
        outs = []
        for t0 in range(0, T, th):
            parts = []
            for g in range(n_groups):
                phi = _from_words(phi_v[i, g * gr:(g + 1) * gr, t0:t0 + th])
                num_den = _dot(_from_words(read_v[g]), phi)
                both = 1.0 / (num_den[gr:gr + 8] + 1e-6)
                swapped = pltpu.roll(both, 4, 0)
                inv0 = jnp.where(first_head, both, swapped)
                inv1 = jnp.where(first_head, swapped, both)
                parts.append(num_den[0:gr] * jnp.concatenate([inv0, inv0, both, inv1, inv1], axis=0))
            outs.append(jnp.concatenate(parts, axis=0).astype(BF16).T)
        o = jnp.concatenate(outs, axis=0)

        hs, hns = [], []
        for r in range(0, T, WO_ROWS):
            hs.append(x_v[i, r:r + WO_ROWS, :].astype(F32) + _dot(o[r:r + WO_ROWS], wo_v[...]))
            hns.append(_layernorm(hs[-1]))
        h = jnp.concatenate(hs, axis=0)
        hn = jnp.concatenate(hns, axis=0)
        hn_ops = [a.astype(BF16) for a in _strassen_lhs(
            hn[0:th, 0:dq], hn[0:th, dq:2 * dq], hn[th:T, 0:dq], hn[th:T, dq:2 * dq])]
        hn_rest = hn[:, 2 * dq:D].astype(BF16)

        acc = None
        act_ops = glu(0, hn_ops, hn_rest)
        for c in range(1, n_chunks):
            nxt = glu(c, hn_ops, hn_rest)
            acc = down(c - 1, act_ops, acc)
            act_ops = nxt
        acc = down(n_chunks - 1, act_ops, acc)
        y11, y12, y21, y22 = _strassen_out(acc[0:7])
        y = h + jnp.concatenate([jnp.concatenate([y11, y12, acc[7][0:th]], axis=1),
                                 jnp.concatenate([y21, y22, acc[7][th:T]], axis=1)], axis=0)
        for u in range(n_out):
            out_v[i * n_out + u] = y[u * OUT_ROWS:(u + 1) * OUT_ROWS].astype(BF16)
            out_copy(i * n_out + u).start()
        return carry

    lax.fori_loop(0, n_tiles, pass2, 0)
    for j in range(n_tiles * n_out):
        out_copy(j).wait()


def build(interpret=False):
    def fn(A_x, A_wqkv, A_w_phi, A_wo, B_x, B_w_gate, B_w_up, B_w_down):
        del B_x
        B, S, D = A_x.shape
        F = B_w_gate.shape[1]
        dh = D // HEADS
        gr = PAIR * dh
        n_tiles = S // TILE
        assert B == 1 and D == 5 * LANES and S % TILE == 0 and n_tiles >= 2 and F % FF_CHUNK == 0
        hbm = pl.BlockSpec(memory_space=pl.ANY)
        out = pl.pallas_call(
            _kernel,
            out_shape=jax.ShapeDtypeStruct((S, D), A_x.dtype),
            in_specs=[hbm] * 7,
            out_specs=hbm,
            scratch_shapes=[
                pltpu.VMEM((n_tiles, TILE, D), BF16),
                pltpu.VMEM((D, D), BF16),
                pltpu.VMEM((WK_SPLIT, D), BF16),
                pltpu.VMEM((D - WK_SPLIT, D), BF16),
                pltpu.VMEM((D, D), BF16),
                pltpu.VMEM((dh, dh, HEADS), BF16),
                pltpu.VMEM((D, D), BF16),
                pltpu.VMEM((D, F), BF16),
                pltpu.VMEM((D, F), BF16),
                pltpu.VMEM((F, D), BF16),
                pltpu.VMEM((D // LANES, 2 * gr, LANES), U32),
                pltpu.VMEM((2, D // 2, D), U32),
                pltpu.VMEM((7, D // 4, 2 * LANES), U32),
                pltpu.VMEM((D // 2, D - 4 * LANES), U32),
                pltpu.VMEM((TILE // 2, D), U32),
                pltpu.VMEM((D, TILE), F32),
                pltpu.VMEM((n_tiles + 1, D, TILE), U32),
                pltpu.VMEM((HEADS // PAIR, gr + 8, 2 * gr), F32),
                pltpu.VMEM((HEADS // PAIR, gr // 2 + 4, 2 * gr), U32),
                pltpu.VMEM((S // OUT_ROWS, OUT_ROWS, D), BF16),
                pltpu.SemaphoreType.DMA((n_tiles,)),
                pltpu.SemaphoreType.DMA((10,)),
                pltpu.SemaphoreType.DMA((S // OUT_ROWS,)),
            ],
            compiler_params=pltpu.CompilerParams(vmem_limit_bytes=100 * 1024 * 1024),
            interpret=interpret,
        )(A_x.reshape(S, D), A_wqkv, A_w_phi.transpose(1, 2, 0), A_wo, B_w_gate, B_w_up, B_w_down)
        return out.reshape(B, S, D)
    return fn


pallas_sequential_preLN__linear_kernel_hedgehog__geglu_ffn__prompt_kernel = jax.jit(build())
```
